```python
import os as _os
_os.environ.setdefault('JAX_PLATFORMS', 'cpu')
import jax
import jax.numpy as jnp

def _softmax(x, axis=-1):
    return jax.nn.softmax(x, axis=axis)

def _gelu(x):
    return jax.nn.gelu(x, approximate=True)

def _silu(x):
    return jax.nn.silu(x)

def _sigmoid(x):
    return jax.nn.sigmoid(x)

def _layernorm(x, axis=-1, eps=1e-05):
    m = jnp.mean(x, axis=axis, keepdims=True)
    v = jnp.var(x, axis=axis, keepdims=True)
    return (x - m) / jnp.sqrt(v + eps)

def _scatter_add(tgt, idx, src, axis=0):
    return tgt.at[idx].add(src)

def _segment_sum(src, seg, n):
    return jax.ops.segment_sum(src, seg, n)

class _Rng:

    def __init__(self, key):
        self._k = key

    def _next(self):
        self._k, sub = jax.random.split(self._k)
        return sub

    def normal(self, shape):
        return jax.random.normal(self._next(), shape, dtype=jnp.bfloat16)

    def randint(self, lo, hi, shape):
        return jax.random.randint(self._next(), shape, lo, hi, dtype=jnp.int32)

    def uniform(self, shape, lo=0.0, hi=1.0):
        return jax.random.uniform(self._next(), shape, jnp.bfloat16, lo, hi)

    def permutation(self, n):
        return jax.random.permutation(self._next(), n)
kernel_name = 'adaLN_cond__compressed_kv_cla__moe_arch_mod__prompt'

def setup_inputs():
    _rng = _Rng(jax.random.key(int.from_bytes(__import__("os").urandom(4), "little")))
    _w = lambda a: (lambda t: t.astype(jnp.bfloat16) if jnp.issubdtype(t.dtype, jnp.floating) else t)(jnp.asarray(a))

    def _A_setup():
        B, H, Sq, Sk, D, M = (1, 32, 2048, 2048, 128, 640)
        Dc = 4 * D
        return {'x': _w((lambda *s: _rng.normal(s) * 0.1)(B, Sq, M)), 'c_kv': _w((lambda *s: _rng.normal(s) * 0.8)(B, Sk, Dc)), 'w_q': _w((lambda *s: _rng.normal(s) * 1.6)(M, H, D) * M ** (-0.5)), 'w_uk': _w((lambda *s: _rng.normal(s) * 1.6)(Dc, H, D) * Dc ** (-0.5)), 'w_uv': _w((lambda *s: _rng.normal(s) * 0.8)(Dc, H, D) * Dc ** (-0.5)), 'w_o': _w((lambda *s: _rng.normal(s) * 0.8)(H, D, M) * (H * D) ** (-0.5))}
    _A_in = _A_setup()

    def _B_setup():
        B, S, D, F, C = (1, 2048, 640, 1728, 8)
        return {'x': _w((lambda *s: _rng.normal(s) * 0.1)(B, S, D)), 'w_r': _w((lambda *s: _rng.normal(s) * 0.1)(D)), 'w_gate': _w((lambda *s: _rng.normal(s) * 0.1)(D, F)), 'w_up': _w((lambda *s: _rng.normal(s) * 0.1)(D, F)), 'w_down': _w((lambda *s: _rng.normal(s) * 0.1)(F, D))}
    _B_in = _B_setup()
    return {'A_x': _A_in['x'], 'A_c_kv': _A_in['c_kv'], 'A_w_q': _A_in['w_q'], 'A_w_uk': _A_in['w_uk'], 'A_w_uv': _A_in['w_uv'], 'A_w_o': _A_in['w_o'], 'B_x': _B_in['x'], 'B_w_r': _B_in['w_r'], 'B_w_gate': _B_in['w_gate'], 'B_w_up': _B_in['w_up'], 'B_w_down': _B_in['w_down'], 'c': _w((lambda *s: _rng.normal(s) * 0.1)(1, 640) * 8.0), 'w_mod': _w((lambda *s: _rng.normal(s) * 0.1)(640, 6 * 640) * 640 ** (-0.5) * 8.0)}

def reference(A_x, A_c_kv, A_w_q, A_w_uk, A_w_uv, A_w_o, B_x, B_w_r, B_w_gate, B_w_up, B_w_down, c, w_mod):

    def _A_ref(x, c_kv, w_q, w_uk, w_uv, w_o):
        B, Sq, M = (x.shape[0], x.shape[1], x.shape[2])
        Sk = c_kv.shape[1]
        H, D = (w_q.shape[1], w_q.shape[2])
        q = jnp.einsum('bqm,mhd->bhqd', x, w_q)
        k = jnp.einsum('bkc,chd->bhkd', c_kv, w_uk)
        v = jnp.einsum('bkc,chd->bhkd', c_kv, w_uv)
        scores = jnp.einsum('bhqd,bhkd->bhqk', q, k) * D ** (-0.5)
        off = Sk - Sq
        qi = jnp.arange(Sq)[:, None]
        kj = jnp.arange(Sk)[None, :]
        cmask = kj <= qi + off
        scores = jnp.where(cmask[None, None], scores, -1000000000.0)
        p = _softmax(scores, axis=-1)
        ctx = jnp.einsum('bhqk,bhkd->bhqd', p, v)
        return jnp.einsum('bhqd,hdm->bqm', ctx, w_o)

    def _B_ref(x, w_r, w_gate, w_up, w_down):
        B, S, D = x.shape
        C = 8
        r = x @ w_r
        idx = jnp.argsort(-r, axis=-1)[:, :C]
        idx_e = jnp.repeat(idx.reshape(B, C, 1), D, axis=2)
        x_sel = jnp.take_along_axis(x, idx_e, axis=1)
        g = _silu(x_sel @ w_gate)
        u = x_sel @ w_up
        y = g * u @ w_down
        r_sel = _sigmoid(jnp.take_along_axis(r, idx, axis=1))
        y = y * r_sel.reshape(B, C, 1)
        b_off = (jnp.arange(B) * S).reshape(B, 1)
        flat_idx = (idx + b_off).reshape(B * C)
        zero = (x * 0.0).reshape(B * S, D)
        upd = _scatter_add(zero, flat_idx, y.reshape(B * C, D), axis=0)
        return x + upd.reshape(B, S, D)
    x = A_x
    mod = (_silu(c) @ w_mod).reshape(c.shape[0], 6, 1, -1)
    sa, ca, ga, sb, cb, gb = (mod[:, 0].copy(), mod[:, 1].copy(), mod[:, 2].copy(), mod[:, 3].copy(), mod[:, 4].copy(), mod[:, 5].copy())
    h = _layernorm(x, axis=-1) * (1 + ca) + sa
    x = x + ga * _A_ref(h, A_c_kv, A_w_q, A_w_uk, A_w_uv, A_w_o)
    h = _layernorm(x, axis=-1) * (1 + cb) + sb
    x = x + gb * _B_ref(h, B_w_r, B_w_gate, B_w_up, B_w_down)
    return x
```

```python
import functools
import jax
import jax.numpy as jnp
from jax import lax
import jax.experimental.pallas as pl
import jax.experimental.pallas.tpu as pltpu

S = 2048
M = 640
DC = 512
H = 32
D = 128
F = 1728
C = 8
TQ = 256
HB = TQ // 2
NB = S // TQ
NP = H // 2
CH = 4
EPS = 1e-5
LOG2E = 1.4426950408889634
NEG = -1e30
QSCALE = (D ** -0.5) * LOG2E
f32 = jnp.float32
bf16 = jnp.bfloat16
u32 = jnp.uint32
NT = (((1,), (1,)), ((), ()))

SEM_W = 0
SEM_WO = 9
SEM_CKV = 11
SEM_X = 13
SEM_C = 15
SEM_MODA = 16
SEM_MODB = 17
SEM_WR = 18
SEM_WG = 19
SEM_WU = 20
SEM_WD = 21
SEM_OUT = 22
SEM_FIX = 30
NSEM = 38


def _bf(x):
    return x.astype(bf16).astype(f32)


def _ln(x):
    m = jnp.mean(x, axis=-1, keepdims=True)
    xc = x - m
    v = jnp.mean(xc * xc, axis=-1, keepdims=True)
    return xc * lax.rsqrt(v + EPS)


def _unpack_pair(w32):
    lo = pltpu.bitcast(w32 << 16, f32).astype(bf16)
    hi = pltpu.bitcast(w32 & jnp.uint32(0xFFFF0000), f32).astype(bf16)
    return lo, hi


def _kernel(x_hbm, ckv_hbm, wq_hbm, wuk_hbm, wuv_hbm, wo_hbm, wr_hbm, wg_hbm, wu_hbm,
            wd_hbm, c_hbm, wmod_hbm, out_hbm,
            x_buf, ckv_buf, h1_ref, acc_ref, mod_ref, k_ref, v_ref, q7_ref,
            wq_buf, wk_buf, wv_buf, wo_buf, wmod_buf, c_buf, wr_buf, wg_buf, wu_buf, wd_buf,
            out_buf, sems):
    def cp(src, dst, s):
        return pltpu.make_async_copy(src, dst, sems.at[s])

    def wq_cp(jj, sl):
        return cp(wq_hbm.bitcast(u32).at[:, jj, :], wq_buf.at[sl], SEM_W + 3 * sl)

    def wkv_cp(jj, sl):
        return [cp(wuk_hbm.bitcast(u32).at[:, jj, :], wk_buf.at[sl], SEM_W + 3 * sl + 1),
                cp(wuv_hbm.bitcast(u32).at[:, jj, :], wv_buf.at[sl], SEM_W + 3 * sl + 2)]

    def wo_cp(jj, sl):
        return cp(wo_hbm.at[pl.ds((jj * (2 * D) if isinstance(jj, int) else pl.multiple_of(jj * (2 * D), 2 * D)), 2 * D), :], wo_buf.at[sl],
                  SEM_WO + sl)

    HS = S // 2

    def ckv_cp(t):
        return cp(ckv_hbm.at[t * HS:(t + 1) * HS, :], ckv_buf.at[t * HS:(t + 1) * HS, :], SEM_CKV + t)

    def x_cp(t):
        return cp(x_hbm.at[t * HS:(t + 1) * HS, :], x_buf.at[t * HS:(t + 1) * HS, :], SEM_X + t)

    c_cp = lambda: cp(c_hbm, c_buf, SEM_C)
    moda_cp = lambda: cp(wmod_hbm.at[:, 0:2 * M], wmod_buf.at[:, 0:2 * M], SEM_MODA)
    modb_cp = lambda: cp(wmod_hbm.at[:, 2 * M:6 * M], wmod_buf.at[:, 2 * M:6 * M], SEM_MODB)
    late_cps = lambda: [modb_cp(), cp(wr_hbm, wr_buf, SEM_WR)]
    ffn_cps = lambda: [cp(wg_hbm, wg_buf, SEM_WG), cp(wu_hbm, wu_buf, SEM_WU), cp(wd_hbm, wd_buf, SEM_WD)]

    def out_cp(i):
        return cp(out_buf.at[i * TQ:(i + 1) * TQ, :], out_hbm.at[i * TQ:(i + 1) * TQ, :], SEM_OUT + i)

    def silu_c():
        c = c_buf[...].astype(f32)
        sc = (c * jax.nn.sigmoid(c)).astype(bf16)
        return jnp.broadcast_to(sc, (8, M))

    def get_wq(sl):
        return jnp.concatenate(_unpack_pair(wq_buf[sl]), axis=1)

    def get_wkv(sl):
        return jnp.concatenate(_unpack_pair(wk_buf[sl]) + _unpack_pair(wv_buf[sl]), axis=1)

    def rows(i):
        return slice(i * TQ, (i + 1) * TQ)

    def qproj(wq, i):
        q = jnp.dot(h1_ref[rows(i), :], wq, preferred_element_type=f32)
        return (q * QSCALE).astype(bf16)

    def kvproj(wkv, i):
        kv = jnp.dot(ckv_buf[rows(i), :], wkv, preferred_element_type=f32)
        for hh in range(2):
            k_ref[hh, rows(i), :] = kv[:, hh * D:(hh + 1) * D].astype(bf16)
            v_ref[hh, rows(i), :] = kv[:, (2 + hh) * D:(3 + hh) * D].astype(bf16)

    for c_ in wkv_cp(0, 0):
        c_.start()
    ckv_cp(0).start()
    ckv_cp(1).start()
    c_cp().start()
    moda_cp().start()
    x_cp(1).start()
    wq_cp(0, 0).start()
    x_cp(0).start()
    for c_ in wkv_cp(1, 1):
        c_.start()
    wq_cp(1, 1).start()
    wo_cp(0, 0).start()

    for c_ in wkv_cp(0, 0):
        c_.wait()
    ckv_cp(0).wait()
    wkv = get_wkv(0)
    acc_ref[...] = jnp.zeros_like(acc_ref)
    for i in range(NB // 2):
        kvproj(wkv, i)
    ckv_cp(1).wait()
    c_cp().wait()
    moda_cp().wait()
    x_cp(1).wait()
    wq_cp(0, 0).wait()
    mod = _bf(jnp.dot(silu_c(), wmod_buf[:, 0:2 * M], preferred_element_type=f32))
    sa = mod[0:1, 0:M]
    ca1 = 1.0 + mod[0:1, M:2 * M]

    def ln1(i):
        x = x_buf[rows(i), :].astype(f32)
        h1_ref[rows(i), :] = (_ln(x) * ca1 + sa).astype(bf16)

    for i in range(NB // 2, NB - 1):
        kvproj(wkv, i)
        ln1(NB - 1 - (i - NB // 2))
    ln1(NB // 2)
    x_cp(0).wait()
    kvproj(wkv, NB - 1)
    q7_ref[...] = qproj(get_wq(0), NB - 1)
    for i in range(NB // 2):
        ln1(i)

    row = lax.broadcasted_iota(jnp.int32, (HB, HB), 0)
    col = lax.broadcasted_iota(jnp.int32, (HB, HB), 1)

    def tiles(x):
        return [x[:, t * 128:(t + 1) * 128] for t in range(x.shape[1] // 128)]

    def scores(q, hh, i):
        tri = col <= row
        qb = q[:, hh * D:(hh + 1) * D]
        nt = 2 * i + 1
        chunks = []
        mrun = None
        for c0 in range(0, nt, CH):
            c1 = min(nt, c0 + CH)
            sc = lax.dot_general(qb, k_ref[hh, c0 * 128:c1 * 128, :], NT, preferred_element_type=f32)
            ts = tiles(sc)
            if c1 == nt:
                last = ts[-1]
                ts[-1] = jnp.concatenate([jnp.where(tri, last[:HB], NEG), last[HB:]], axis=0)
            for t in ts:
                mrun = t if mrun is None else jnp.maximum(mrun, t)
            chunks.append(ts)
        L = nt * 128
        s_ext = lax.dot_general(qb[HB:], k_ref[hh, L:L + HB, :], NT, preferred_element_type=f32)
        s_ext = jnp.where(tri, s_ext, NEG)
        mrun = jnp.concatenate([mrun[:HB], jnp.maximum(mrun[HB:], s_ext)], axis=0)
        m = jnp.max(mrun, axis=-1, keepdims=True)
        return chunks, s_ext, m

    def pv(s, hh, i):
        chunks, s_ext, m = s
        mb = jnp.broadcast_to(m, (TQ, 128))
        lrun = None
        o = None
        c0 = 0
        for ts in chunks:
            ps = [jnp.exp2(t - mb) for t in ts]
            for p in ps:
                lrun = p if lrun is None else lrun + p
            pc = jnp.concatenate(ps, axis=1).astype(bf16)
            oc = jnp.dot(pc, v_ref[hh, c0 * 128:(c0 + len(ts)) * 128, :], preferred_element_type=f32)
            o = oc if o is None else o + oc
            c0 += len(ts)
        L = c0 * 128
        p_ext = jnp.exp2(s_ext - mb[HB:])
        o_ext = jnp.dot(p_ext.astype(bf16), v_ref[hh, L:L + HB, :], preferred_element_type=f32)
        lrun = jnp.concatenate([lrun[:HB], lrun[HB:] + p_ext], axis=0)
        o = jnp.concatenate([o[:HB], o[HB:] + o_ext], axis=0)
        l = jnp.sum(lrun, axis=-1, keepdims=True)
        return (o * (1.0 / l)).astype(bf16)

    def step(j, last):
        sl = j % 3
        sln = (j + 1) % 3
        slo = j % 2
        wo_cp(j, slo).wait()
        if not last:
            wo_cp(j + 1, 1 - slo).start()
            wq_cp(j + 1, sln).wait()
            for c_ in wkv_cp(j + 1, sln):
                c_.wait()

            @pl.when(j == 1)
            def _():
                for c_ in late_cps() + ffn_cps():
                    c_.start()

            @pl.when(j + 2 < NP)
            def _():
                sl2 = (j + 2) % 3
                wq_cp(j + 2, sl2).start()
                for c_ in wkv_cp(j + 2, sl2):
                    c_.start()
        else:
            for c_ in late_cps():
                c_.wait()

        wq = get_wq(sl)
        if not last:
            wkv_n = get_wkv(sln)
        else:
            mod = _bf(jnp.dot(silu_c(), wmod_buf[:, 2 * M:6 * M], preferred_element_type=f32))
            mod_ref[...] = mod
            ga = mod[0:1, 0:M]
            sb = mod[0:1, M:2 * M]
            cb1 = _bf(1.0 + mod[0:1, 2 * M:3 * M])
            gb = mod[0:1, 3 * M:4 * M]
            wr8 = jnp.broadcast_to(wr_buf[...], (8, M))
            sub8 = lax.broadcasted_iota(jnp.int32, (8, TQ), 0)
            rall = [jnp.zeros((8, TQ), f32)]

        def oproj(ctx, i):
            a = acc_ref[rows(i), :] + jnp.dot(ctx, wo_buf[slo], preferred_element_type=f32)
            if not last:
                acc_ref[rows(i), :] = a
            else:
                x1 = _bf(x_buf[rows(i), :].astype(f32) + ga * a)
                acc_ref[rows(i), :] = x1
                h2 = (_ln(x1) * cb1 + sb).astype(bf16)
                out_buf[rows(i), :] = (x1 + gb * h2.astype(f32)).astype(bf16)
                out_cp(i).start()
                rb = lax.dot_general(wr8, h2, NT, preferred_element_type=f32)
                rall[0] = jnp.where(sub8 == i, rb, rall[0])

        qs = {NB - 1: q7_ref[...]}
        ctx = {}
        for i in range(NB - 1, -1, -1):
            sA = scores(qs[i], 0, i)
            if i == NB - 1:
                qs[i - 1] = qproj(wq, i - 1)
            elif not last:
                kvproj(wkv_n, i + 1)
            elif i >= 2:
                qs[i - 2] = qproj(wq, i - 2)
            if not (last and i < 2):
                cA = pv(sA, 0, i)
            sB = scores(qs[i], 1, i)
            if i + 1 in ctx:
                oproj(ctx.pop(i + 1), i + 1)
            if i >= 2 and (not last or i == NB - 1):
                qs[i - 2] = qproj(wq, i - 2)
            if last and i < 2:
                cA = pv(sA, 0, i)
            cB = pv(sB, 1, i)
            ctx[i] = jnp.concatenate([cA, cB], axis=1)
        if not last:
            kvproj(wkv_n, 0)
            q7_ref[...] = qproj(get_wq(sln), NB - 1)
        oproj(ctx.pop(0), 0)

        if last:
            r = _bf(rall[0])
            rb = pltpu.bitcast(r, jnp.int32)
            key = jnp.where(rb < 0, rb ^ jnp.int32(0x7FFF0000), rb)
            idx = sub8 * TQ + lax.broadcasted_iota(jnp.int32, (8, TQ), 1)
            key = (key & jnp.int32(-65536)) | (S - 1 - idx)
            sel_idx = []
            for t in range(C):
                kmax = jnp.max(key)
                it = S - 1 - (kmax & 0xFFFF)
                sel_idx.append(it)
                key = jnp.where(key == kmax, jnp.int32(-2 ** 31), key)
            for c_ in ffn_cps():
                c_.wait()
            x1s = jnp.concatenate([acc_ref[pl.ds(it, 1), :] for it in sel_idx], axis=0)
            xsb = (_ln(x1s) * cb1 + sb).astype(bf16)
            xs = xsb.astype(f32)
            rs = _bf(jnp.sum(xs * wr_buf[...].astype(f32), axis=-1, keepdims=True))
            g = _bf(lax.dot_general(xsb, wg_buf[...], NT, preferred_element_type=f32))
            g = _bf(g * jax.nn.sigmoid(g))
            u = _bf(lax.dot_general(xsb, wu_buf[...], NT, preferred_element_type=f32))
            y = _bf(jnp.dot((g * u).astype(bf16), wd_buf[...], preferred_element_type=f32))
            y = _bf(y * _bf(jax.nn.sigmoid(rs)))
            newrows = x1s + _bf(gb * _bf(xs + y))
            for i in range(NB):
                out_cp(i).wait()
            sub = lax.broadcasted_iota(jnp.int32, (16, M), 0)
            bases = []
            for t in range(C):
                it = sel_idx[t]
                base = pl.multiple_of((it >> 4) << 4, 16)
                bases.append(base)
                cur = out_buf[pl.ds(base, 16), :].astype(f32)
                out_buf[pl.ds(base, 16), :] = jnp.where(sub == (it & 15), newrows[t:t + 1, :], cur).astype(bf16)

            def fix_cp(t):
                return cp(out_buf.at[pl.ds(bases[t], 16), :], out_hbm.at[pl.ds(bases[t], 16), :], SEM_FIX + t)

            uniq = []
            for t in range(C):
                u_ = jnp.bool_(True)
                for t2 in range(t):
                    u_ = jnp.logical_and(u_, bases[t] != bases[t2])
                uniq.append(u_)
            for t in range(C):
                @pl.when(uniq[t])
                def _():
                    fix_cp(t).start()
            for t in range(C):
                @pl.when(uniq[t])
                def _():
                    fix_cp(t).wait()

    def body(j, carry):
        with jax.named_scope("main"):
            step(j, False)
        return carry

    lax.fori_loop(0, NP - 1, body, 0)
    with jax.named_scope("last"):
        step(NP - 1, True)


@jax.jit
def pallas_adaLN_cond__compressed_kv_cla__moe_arch_mod__prompt_kernel(
    A_x, A_c_kv, A_w_q, A_w_uk, A_w_uv, A_w_o, B_x, B_w_r, B_w_gate, B_w_up, B_w_down, c, w_mod,
):
    x = A_x.reshape(S, M)
    ckv = A_c_kv.reshape(S, DC)
    wo = A_w_o.reshape(H * D, M)
    wr = B_w_r.reshape(1, M)
    hbm = pl.BlockSpec(memory_space=pltpu.HBM)

    out = pl.pallas_call(
        _kernel,
        in_specs=[hbm] * 12,
        out_specs=hbm,
        out_shape=jax.ShapeDtypeStruct((S, M), bf16),
        scratch_shapes=[
            pltpu.VMEM((S, M), bf16),
            pltpu.VMEM((S, DC), bf16),
            pltpu.VMEM((S, M), bf16),
            pltpu.VMEM((S, M), f32),
            pltpu.VMEM((8, 4 * M), f32),
            pltpu.VMEM((2, S, D), bf16),
            pltpu.VMEM((2, S, D), bf16),
            pltpu.VMEM((TQ, 2 * D), bf16),
            pltpu.VMEM((3, M, D), u32),
            pltpu.VMEM((3, DC, D), u32),
            pltpu.VMEM((3, DC, D), u32),
            pltpu.VMEM((2, 2 * D, M), bf16),
            pltpu.VMEM((M, 6 * M), bf16),
            pltpu.VMEM((1, M), bf16),
            pltpu.VMEM((1, M), bf16),
            pltpu.VMEM((F, M), bf16),
            pltpu.VMEM((F, M), bf16),
            pltpu.VMEM((F, M), bf16),
            pltpu.VMEM((S, M), bf16),
            pltpu.SemaphoreType.DMA((NSEM,)),
        ],
        compiler_params=pltpu.CompilerParams(
            vmem_limit_bytes=100 * 1024 * 1024,
        ),
    )(x, ckv, A_w_q, A_w_uk, A_w_uv, wo, wr, B_w_gate.T, B_w_up.T, B_w_down, c, w_mod)
    return out.reshape(1, S, M)
```

```python
import jax
import jax.numpy as jnp
from jax import lax
import jax.experimental.pallas as pl
import jax.experimental.pallas.tpu as pltpu

S = 2048
M = 640
DC = 512
H = 32
D = 128
F = 1728
C = 8
TQ = 256
HB = TQ // 2
NB = S // TQ
NP = H // 2
PR = 16
EPS = 1e-5
LOG2E = 1.4426950408889634
NEG = -1e30
QSCALE = (D ** -0.5) * LOG2E
f32 = jnp.float32
bf16 = jnp.bfloat16
u32 = jnp.uint32
i32 = jnp.int32
NT = (((1,), (1,)), ((), ()))

SEM_WQ = 0
SEM_WV = 4
SEM_WO = 8
SEM_GU = 10
SEM_CKV = 14
SEM_X = 18
SEM_C = 20
SEM_MODA = 21
SEM_MODB = 22
SEM_WR = 23
SEM_WD = 24
SEM_OUT = 25
SEM_FIX = 33
SEM_WK = 41
NSEM = 45

NST = 14
LAST0 = F - 128
CKV_CHUNKS = ((0, 1), (1, 3), (3, 6), (6, 8))
X_CHUNKS = ((5, 8), (0, 5))
S_CHUNK = 3
PAD_ROWS = 1000


def _bf(x):
    return x.astype(bf16).astype(f32)


def _unpack_pair(w32):
    lo = pltpu.bitcast(w32 << 16, f32).astype(bf16)
    hi = pltpu.bitcast(w32 & jnp.uint32(0xFFFF0000), f32).astype(bf16)
    return lo, hi


def _b16(x32):
    return pltpu.bitcast(x32, bf16)


def _p32(x16):
    return pltpu.bitcast(x16, u32)


def _tiles(x):
    return [x[:, t * 128:(t + 1) * 128] for t in range(x.shape[1] // 128)]


def _cat0(*xs):
    return jnp.concatenate(xs, axis=0)


def _cat1(*xs):
    return jnp.concatenate(xs, axis=1)


def _bc(v):
    return jnp.broadcast_to(v, (v.shape[0], 128))


def _rep(v):
    return jnp.concatenate([v] * (M // 128), axis=1)


def _bits(v):
    x32 = pltpu.bitcast(v, u32)
    dep = None
    for g in range(x32.shape[0] // 8):
        for t in _tiles(x32[8 * g:8 * g + 8]):
            dep = t if dep is None else dep | t
    return dep


def _anchor(x16, deps):
    if not deps:
        return x16
    x32 = _p32(x16)
    parts = []
    for g in range(x32.shape[0] // 8):
        r = x32[8 * g:8 * g + 8]
        if g in deps:
            t = r[:, :128]
            t = t & (t | deps[g])
            r = t if r.shape[1] == 128 else _cat1(t, r[:, 128:])
        parts.append(r)
    return _b16(jnp.concatenate(parts, axis=0))


def _gate(x, tok):
    if tok is None:
        return x
    t = pltpu.bitcast(x[:, :128], u32)
    t = t & (t | jnp.concatenate([tok] * (x.shape[0] // 8), axis=0))
    t = pltpu.bitcast(t, x.dtype)
    return t if x.shape[1] == 128 else _cat1(t, x[:, 128:])


def _normalize(o, lrun):
    l = jnp.sum(lrun, axis=-1, keepdims=True)
    rc = pl.reciprocal(l, approx=True)
    rc = rc * (2.0 - l * rc)
    return (o * rc).astype(bf16)


def _kernel(x_hbm, ckv_hbm, wq_hbm, wuk_hbm, wuv_hbm, wo_hbm, wr_hbm, wg_hbm, wu_hbm,
            wd_hbm, c_hbm, wmod_hbm, out_hbm,
            x_buf, ckv_buf, h1_ref, acc_ref, k_ref, v_ref, q_ref,
            wq_buf, wk_buf, wv_buf, wo_buf, wmod_buf, c_buf, wr_buf, gu_buf, gu_t, wd_buf,
            out_buf, eye_ref, st_ref, sems):

    def cp(src, dst, s):
        return pltpu.make_async_copy(src, dst, sems.at[s])

    def wq_cp(jj):
        sl = jj & 3
        return cp(wq_hbm.bitcast(u32).at[:, jj, :], wq_buf.at[sl], SEM_WQ + sl)

    def wkv_cp(jj):
        sl = jj & 3
        return [cp(wuk_hbm.bitcast(u32).at[:, jj, :], wk_buf.at[sl], SEM_WK + sl),
                cp(wuv_hbm.bitcast(u32).at[:, jj, :], wv_buf.at[sl], SEM_WV + sl)]

    def wo_cp(part):
        r0, r1 = (0, D) if part == 0 else (D, NP * D)
        return cp(wo_hbm.bitcast(u32).at[r0:r1, :], wo_buf.at[r0:r1, :], SEM_WO + part)

    def ckv_cp(t):
        a, b = CKV_CHUNKS[t]
        return cp(ckv_hbm.bitcast(u32).at[a * HB:b * HB, :], ckv_buf.at[a * HB:b * HB, :], SEM_CKV + t)

    def x_cp(t):
        a, b = X_CHUNKS[t]
        return cp(x_hbm.bitcast(u32).at[a * HB:b * HB, :], x_buf.at[a * HB:b * HB, :], SEM_X + t)

    def c_cp():
        return cp(c_hbm, c_buf, SEM_C)

    def moda_cp():
        return cp(wmod_hbm.bitcast(u32).at[:, 0:2 * M], wmod_buf.at[:, 0:2 * M], SEM_MODA)

    def late_cps():
        return [cp(wmod_hbm.bitcast(u32).at[:, 2 * M:6 * M], wmod_buf.at[:, 2 * M:6 * M], SEM_MODB),
                cp(wr_hbm, wr_buf, SEM_WR),
                cp(wd_hbm.bitcast(u32), wd_buf, SEM_WD)]

    def gu_cp(part):
        r0, r1 = (0, 64) if part == 0 else (64, F // 2)
        return [cp(w.bitcast(u32).at[r0:r1, :], gu_buf.at[n, r0:r1, :], SEM_GU + 2 * part + n)
                for n, w in enumerate((wg_hbm, wu_hbm))]

    def out_cp(i):
        return cp(out_buf.at[i * TQ:(i + 1) * TQ, :], out_hbm.at[i * TQ:(i + 1) * TQ, :], SEM_OUT + i)

    def silu_c():
        c = c_buf[...].astype(f32)
        sc = (c * jax.nn.sigmoid(c)).astype(bf16)
        return jnp.broadcast_to(sc, (8, M))

    def get_wq(jj):
        return jnp.concatenate(_unpack_pair(wq_buf[jj & 3]), axis=1)

    def get_wkv(jj):
        return jnp.concatenate(_unpack_pair(wk_buf[jj & 3]) + _unpack_pair(wv_buf[jj & 3]), axis=1)

    def get_wo(jj):
        st = jj * D if isinstance(jj, int) else pl.multiple_of(jj * D, D)
        return _b16(wo_buf[pl.ds(st, D), :])

    def kv_refs(jj):
        sl = jj & 1
        return k_ref.at[sl], v_ref.at[sl]

    def rows(i):
        return slice(i * TQ, (i + 1) * TQ)

    def hrows(i):
        return slice(i * HB, (i + 1) * HB)

    clock = [0]
    hooks = {'take': None, 'post': None}

    def post(res, dur):
        if hooks['post']:
            hooks['post'](res, dur)

    def take(ng):
        return hooks['take'](ng) if hooks['take'] else {}

    def qproj(wq, i, r0=0, r1=TQ):
        h = _b16(h1_ref[i * HB + r0 // 2:i * HB + r1 // 2, :])
        q = jnp.dot(h, wq, preferred_element_type=f32)
        clock[0] += (r1 - r0) * 5 * (wq.shape[1] // D) // 4
        return (q * QSCALE).astype(bf16)

    def qstore(wq, i, r0=0, r1=TQ):
        q_ref[i * HB + r0 // 2:i * HB + r1 // 2, :] = _p32(qproj(wq, i, r0, r1))

    def qload(i):
        return _b16(q_ref[hrows(i), :])

    def kvproj(wkv, kvr, i):
        kr, vr = kvr
        kv = _tiles(jnp.dot(_b16(ckv_buf[hrows(i), :]), wkv, preferred_element_type=f32))
        for hh in range(2):
            kr[hh, hrows(i), :] = _p32(kv[hh].astype(bf16))
            vr[hh, hrows(i), :] = _p32(kv[2 + hh].astype(bf16))

    row = lax.broadcasted_iota(i32, (HB, HB), 0)
    col = lax.broadcasted_iota(i32, (HB, HB), 1)

    def scores(q, kvr, hh, i):
        kr = kvr[0]
        tri = col <= row
        qb = q[:, hh * D:(hh + 1) * D]
        nt = 2 * i + 1
        tiles = []
        mrun = None
        for c0 in range(0, nt, S_CHUNK):
            c1 = min(nt, c0 + S_CHUNK)
            sc = lax.dot_general(_anchor(qb, take(4 * (c1 - c0))), _b16(kr[hh, c0 * 64:c1 * 64, :]), NT,
                                 preferred_element_type=f32)
            post(sc, 64 * (c1 - c0))
            clock[0] += 64 * (c1 - c0)
            ts = _tiles(sc)
            if c1 == nt:
                last = ts[-1]
                ts[-1] = _cat0(jnp.where(tri, last[:HB], NEG), last[HB:])
            for t in ts:
                mrun = t if mrun is None else jnp.maximum(mrun, t)
            tiles += ts
        s_ext = lax.dot_general(qb[HB:], _b16(kr[hh, nt * 64:(nt + 1) * 64, :]), NT,
                                preferred_element_type=f32)
        clock[0] += 32
        s_ext = jnp.where(tri, s_ext, NEG)
        mrun = _cat0(mrun[:HB], jnp.maximum(mrun[HB:], s_ext))
        m = jnp.max(mrun, axis=-1, keepdims=True)
        return tiles, s_ext, m

    def pv(s, kvr, hh, chunk=2, tie=False):
        vr = kvr[1]
        tiles, s_ext, m = s
        mb = jnp.broadcast_to(m, (TQ, 128))
        lrun = None
        o = None
        for c0 in range(0, len(tiles), chunk):
            ps = [jnp.exp2(t - mb) for t in tiles[c0:c0 + chunk]]
            for p in ps:
                lrun = p if lrun is None else lrun + p
            if tie and lrun is not ps[-1]:
                ps[-1] = jnp.minimum(ps[-1], lrun)
            pc = jnp.concatenate(ps, axis=1).astype(bf16)
            pc = _anchor(pc, take(4 * len(ps)))
            oc = jnp.dot(pc, _b16(vr[hh, c0 * 64:(c0 + len(ps)) * 64, :]), preferred_element_type=f32)
            o = oc if o is None else o + oc
            clock[0] += 64 * len(ps)
        nt = len(tiles)
        p_ext = jnp.exp2(s_ext - mb[HB:])
        o_ext = jnp.dot(p_ext.astype(bf16), _b16(vr[hh, nt * 64:(nt + 1) * 64, :]),
                        preferred_element_type=f32)
        post(o_ext, 128)
        clock[0] += 32
        lrun = _cat0(lrun[:HB], lrun[HB:] + p_ext)
        o = _cat0(o[:HB], o[HB:] + o_ext)
        return _normalize(o, lrun)

    def pv_rows(s, kvr, hh, r0, r1, rel):
        vr = kvr[1]
        tiles, s_ext, m = s
        ts_all = [t[r0:r1] for t in tiles]
        if r0 >= HB:
            ts_all.append(s_ext[r0 - HB:r1 - HB])
        mb = _gate(jnp.broadcast_to(m[r0:r1], (r1 - r0, 128)), rel)
        lrun = None
        o = None
        tok = None
        for c0 in range(0, len(ts_all), 4):
            ps = [jnp.exp2(t - mb) for t in ts_all[c0:c0 + 4]]
            for p in ps:
                lrun = p if lrun is None else lrun + p
            pc = jnp.concatenate(ps, axis=1).astype(bf16)
            oc = jnp.dot(pc, _b16(vr[hh, c0 * 64:(c0 + len(ps)) * 64, :]), preferred_element_type=f32)
            o = oc if o is None else o + oc
            if c0 == 0:
                tok = pltpu.bitcast(oc[0:8], u32)
        return _normalize(o, lrun), tok

    def prologue():
        first = ([ckv_cp(0)] + wkv_cp(0) + [ckv_cp(t) for t in range(1, 4)] + wkv_cp(1)
                 + [c_cp(), moda_cp(), x_cp(0), wq_cp(0), x_cp(1), wq_cp(1), wo_cp(0)]
                 + gu_cp(0) + wkv_cp(2) + [wq_cp(2)] + wkv_cp(3) + [wo_cp(1)] + gu_cp(1) + late_cps())
        for c_ in first:
            c_.start()
        acc_ref[...] = jnp.zeros_like(acc_ref)
        eye_ref[...] = jnp.where(col == row, -1, 0).astype(i32)
        h1_ref[0:PAD_ROWS, :] = jnp.zeros((PAD_ROWS, M), u32)

        for c_ in wkv_cp(0):
            c_.wait()
        ckv_cp(0).wait()
        wkv = get_wkv(0)
        kvr = kv_refs(0)
        kvproj(wkv, kvr, 0)
        ckv_cp(1).wait()
        kvproj(wkv, kvr, 1)
        kvproj(wkv, kvr, 2)
        ckv_cp(2).wait()
        for i in range(3, 6):
            kvproj(wkv, kvr, i)
        ckv_cp(3).wait()
        for c_ in wkv_cp(1):
            c_.wait()
        kvproj(wkv, kvr, 6)
        kvproj(wkv, kvr, 7)
        wkv = get_wkv(1)
        kvr = kv_refs(1)
        for i in range(5):
            kvproj(wkv, kvr, i)
        c_cp().wait()
        moda_cp().wait()
        x_cp(0).wait()
        wq_cp(0).wait()
        mod = _bf(jnp.dot(silu_c(), _b16(wmod_buf[:, 0:2 * M]), preferred_element_type=f32))
        sa = mod[0:1, 0:M]
        ca1 = 1.0 + mod[0:1, M:2 * M]
        wq = get_wq(0)

        def ln1q(i, split=False):
            for r0 in range(i * TQ, (i + 1) * TQ, PR):
                x = _b16(x_buf[r0 // 2:(r0 + PR) // 2, :]).astype(f32)
                xc = x - _rep(_bc(jnp.sum(x, axis=-1, keepdims=True)) * (1.0 / M))
                sv = _bc(jnp.sum(xc * xc, axis=-1, keepdims=True))
                rstd = lax.rsqrt(sv * (1.0 / M) + EPS)
                h1_ref[r0 // 2:(r0 + PR) // 2, :] = _p32((xc * _rep(rstd) * ca1 + sa).astype(bf16))
            for r0, r1 in (((0, HB), (HB, TQ)) if split else ((0, TQ),)):
                qstore(wq, i, r0, r1)

        kvproj(wkv, kvr, 5)
        ln1q(7)
        ln1q(6)
        ln1q(5, True)
        x_cp(1).wait()
        kvproj(wkv, kvr, 6)
        ln1q(4)
        kvproj(wkv, kvr, 7)
        ln1q(3)
        ln1q(2)
        ln1q(1)
        ln1q(0, True)
        wq_cp(1).wait()
        wo_cp(0).wait()
        for c_ in wkv_cp(2) + gu_cp(0):
            c_.wait()

    def body(j, carry):
        @pl.when(j + 3 < NP)
        def _():
            wq_cp(j + 3).start()

        @pl.when(j + 4 < NP)
        def _():
            for c_ in wkv_cp(j + 4):
                c_.start()

        wq_n = get_wq(j + 1)
        wkv_n = get_wkv(j + 2)
        kvr = kv_refs(j)

        def oproj(ctx, i):
            acc_ref[rows(i), :] += jnp.dot(ctx, get_wo(j), preferred_element_type=f32)

        def kvhalf(i, n):
            kv = _tiles(jnp.dot(_b16(ckv_buf[hrows(i), :]), wkv_n[:, n * 2 * D:(n + 1) * 2 * D],
                                preferred_element_type=f32))
            for hh in range(2):
                kvr[n][hh, hrows(i), :] = _p32(kv[hh].astype(bf16))

        qs = {}

        def qnext(i):
            if i >= 0:
                if i not in qs:
                    qs[i] = qload(i)
                qstore(wq_n, i)

        qs[NB - 1] = qload(NB - 1)
        prev = None
        for i in range(NB - 1, -1, -1):
            top = i == NB - 1
            s_a = scores(qs[i], kvr, 0, i)
            if top:
                qnext(i)
            else:
                qnext(i - 1)
                kvhalf(i + 1, 0)
            c_a = pv(s_a, kvr, 0, 2, True)
            s_b = scores(qs[i], kvr, 1, i)
            if top:
                qnext(i - 1)
            else:
                kvhalf(i + 1, 1)
                oproj(prev, i + 1)
            c_b = pv(s_b, kvr, 1, 4 if top else 2, True)
            prev = _cat1(c_a, c_b)
        kvproj(wkv_n, kvr, 0)
        oproj(prev, 0)
        for n in range(2):
            r0 = pl.multiple_of(jnp.minimum(j * 64, LAST0 // 2), 32)
            gu_t[j, n] = _p32(_b16(gu_buf[n, pl.ds(r0, 64), :]).T)

        wq_cp(j + 2).wait()

        @pl.when(j == 0)
        def _():
            for c_ in [wo_cp(1)] + gu_cp(1):
                c_.wait()

        @pl.when(j + 3 < NP)
        def _():
            for c_ in wkv_cp(j + 3):
                c_.wait()
        return carry

    def final():
        ja, jb = NP - 2, NP - 1
        for c_ in late_cps():
            c_.wait()
        wq15 = get_wq(jb)
        kvrs = (kv_refs(ja), kv_refs(jb))
        wo2 = _cat0(get_wo(ja), get_wo(jb))
        mods = {}
        wr1 = wr_buf[...].astype(f32).reshape(1, M)
        sub8 = lax.broadcasted_iota(i32, (8, 128), 0)
        lane8 = lax.broadcasted_iota(i32, (8, 128), 1)
        sc8 = silu_c()

        def modq(n):
            w = _b16(wmod_buf[:, (2 + n) * M:(3 + n) * M])
            mods[n] = _bf(jnp.dot(sc8, w, preferred_element_type=f32))[0:1, :]
            clock[0] += 100
            if n == 3:
                mods['ga'] = mods[0]
                mods['sb'] = sb = mods[1]
                mods['cb1'] = cb1 = _bf(1.0 + mods[2])
                mods['gb'] = gb = mods[3]
                mods['gc'] = gb * cb1
                mods['gs'] = gb * sb
                mods['wc'] = wr1 * cb1
                mods['r0'] = jnp.sum(wr1 * sb, axis=-1, keepdims=True)

        def q_mod(i, half, n):
            r0 = half * HB
            qa = qproj(wq15[:, :D], i, r0, r0 + HB)
            modq(n)
            qb = qproj(wq15[:, D:], i, r0, r0 + HB)
            return _cat1(qa, qb)

        cols = []
        state = [(-(2 ** 27)) + sub8]
        done_rows = {}

        def subsum(v, op):
            for sh in (4, 2, 1):
                v = op(v, pltpu.roll(v, sh, 0))
            return v

        def merge(pend):
            kc = jnp.concatenate(pend, axis=0)
            st = state[0]
            gs = [kc[8 * g:8 * g + 8] for g in range(16)]
            r1 = None
            for g, kg in enumerate(gs):
                t = kg & eye_ref[8 * g:8 * g + 8, :]
                r1 = t if r1 is None else r1 | t
            r1 = subsum(r1, jnp.bitwise_or)
            r2 = jnp.where(lane8 < 8, subsum(st & eye_ref[0:8, :], jnp.bitwise_or), -(2 ** 28))
            hi = 0.0
            lo = 0.0
            for rr in (r1, r2):
                cnt = None
                for kg in gs + [st]:
                    t = (rr - kg) >> 31
                    cnt = t if cnt is None else cnt + t
                sel = subsum(cnt, jnp.add) + sub8 == 0
                hi = hi + jnp.where(sel, (rr >> 11).astype(f32), 0.0)
                lo = lo + jnp.where(sel, (rr & 2047).astype(f32), 0.0)
            hi = _bc(jnp.sum(hi, axis=-1, keepdims=True)).astype(i32)
            lo = _bc(jnp.sum(lo, axis=-1, keepdims=True)).astype(i32)
            state[0] = (hi << 11) | lo
            return pltpu.bitcast(state[0], u32)

        def piece(r0):
            rel = yield
            x1 = acc_ref[r0:r0 + PR, :]
            sm = _bc(jnp.sum(_gate(x1, rel), axis=-1, keepdims=True))
            rel = yield
            m = _gate(sm, rel) * (1.0 / M)
            xc = x1 - _rep(m)
            sv = _bc(jnp.sum(xc * xc, axis=-1, keepdims=True))
            rw = _bc(jnp.sum(xc * mods['wc'], axis=-1, keepdims=True))
            rel = yield
            rstd = lax.rsqrt(_gate(sv, rel) * (1.0 / M) + EPS)
            st_ref[r0:r0 + PR, :] = _cat1(m, rstd)
            of = x1 + (xc * _rep(rstd)) * mods['gc'] + mods['gs']
            out_buf[r0:r0 + PR, :] = of.astype(bf16)
            blk = r0 // TQ
            done_rows[blk] = done_rows.get(blk, 0) + PR
            if done_rows[blk] == TQ:
                out_cp(blk).start()
            r = _bf(rw * rstd + mods['r0'])
            rb = pltpu.bitcast(r, i32) >> 16
            rb = rb ^ ((rb >> 31) & 0x7FFF)
            idx = (S - 1 - r0) - lax.broadcasted_iota(i32, (PR, 128), 0)
            key = (rb << 11) | idx
            cols.append(key)
            return _bits(of) | _bits(key)

        def merge_task(pend):
            rel = yield
            return merge([_gate(pend[0], rel)] + pend[1:])

        live = []
        anchors = []
        nxt = [0]
        stage_gap = 200
        stage_cost = (48, 32, 48, 96)

        def advance(ent, t, rel):
            try:
                ent[2].send(rel)
                ent[0] = t + stage_gap
                ent[1] += 1
            except StopIteration as e:
                anchors.append([t + (470 if ent[1] == 3 else 320), e.value])
                live.remove(ent)
                if len(cols) * PR == 128:
                    g = merge_task(list(cols))
                    del cols[:]
                    next(g)
                    live.insert(0, [t + stage_gap, 3, g])

        def post_impl(res, dur):
            for g in range(min(res.shape[0] // 16, dur // 16)):
                t = clock[0] + 16 * g
                if t < nxt[0]:
                    continue
                for ent in live:
                    if ent[0] <= t:
                        nxt[0] = t + stage_cost[ent[1]]
                        advance(ent, t, pltpu.bitcast(res[16 * g:16 * g + 8, 0:128], u32))
                        break

        def take_impl(ng):
            deps = {}
            for g in range(ng):
                t = clock[0] + 16 * g
                ready = [an for an in anchors if an[0] <= t]
                anchors[:] = [an for an in anchors if an[0] > t]
                for an in ready:
                    deps[g] = an[1] | deps[g] if g in deps else an[1]
            return deps

        def ofin(ctx, i, r0, r1, w):
            rs = slice(i * TQ + r0, i * TQ + r1)
            lhs = _anchor(ctx, take((r1 - r0) // 16))
            a = acc_ref[rs, :] + jnp.dot(lhs, w, preferred_element_type=f32)
            clock[0] += 5 * (r1 - r0) * w.shape[0] // 512
            x = _b16(x_buf[(i * TQ + r0) // 2:(i * TQ + r1) // 2, :]).astype(f32)
            acc_ref[rs, :] = x + mods['ga'] * a
            for r in range(i * TQ + r0, i * TQ + r1, PR):
                g = piece(r)
                next(g)
                live.append([clock[0], 0, g])

        def opart(ctx, i, r0, r1):
            rs = slice(i * TQ + r0, i * TQ + r1)
            lhs = _anchor(ctx[r0:r1], take((r1 - r0) // 16))
            acc_ref[rs, :] += jnp.dot(lhs, wo2[:2 * D], preferred_element_type=f32)
            clock[0] += 5 * (r1 - r0) // 2

        hooks.update(take=take_impl, post=post_impl)
        clock[0] = 0
        q15 = {}
        prev = None
        for i in range(NB):
            q14 = qload(i)
            lastb = i == NB - 1
            oprev = lambda r0, r1: ofin(prev[r0:r1], i - 1, r0, r1, wo2)
            if i < 2:
                s_a = scores(q14, kvrs[0], 0, i)
                s_b = scores(q14, kvrs[0], 1, i)
                if i == 0:
                    q15[0] = _cat0(q_mod(0, 0, 0), q_mod(0, 1, 1))
                else:
                    oprev(0, 192)
                c_a = pv(s_a, kvrs[0], 0)
                c_b = pv(s_b, kvrs[0], 1)
                s_c = scores(q15[i], kvrs[1], 0, i)
                s_d = scores(q15[i], kvrs[1], 1, i)
                if i == 0:
                    q15[1] = _cat0(q_mod(1, 0, 2), q_mod(1, 1, 3))
                else:
                    oprev(192, TQ)
                    q15[i + 1] = qproj(wq15, i + 1)
                c_c = pv(s_c, kvrs[1], 0)
                c_d = pv(s_d, kvrs[1], 1)
            else:
                s_a = scores(q14, kvrs[0], 0, i)
                oprev(0, 96)
                c_a = pv(s_a, kvrs[0], 0)
                s_b = scores(q14, kvrs[0], 1, i)
                oprev(96, 192)
                c_b = pv(s_b, kvrs[0], 1)
                s_c = scores(q15[i], kvrs[1], 0, i)
                oprev(192, TQ)
                if lastb:
                    c_ab = _cat1(c_a, c_b)
                    opart(c_ab, i, 0, 64)
                else:
                    qa = qproj(wq15, i + 1, 0, 64)
                c_c = pv(s_c, kvrs[1], 0)
                s_d = scores(q15[i], kvrs[1], 1, i)
                if lastb:
                    opart(c_ab, i, 64, TQ)
                    break
                q15[i + 1] = _cat0(qa, qproj(wq15, i + 1, 64, TQ))
                c_d = pv(s_d, kvrs[1], 1)
            prev = _cat1(c_a, c_b, c_c, c_d)
        hooks.update(take=None, post=None)
        rq = 64
        parts = []
        tok = None
        for k in range(TQ // rq + 1):
            if k < TQ // rq:
                part, tok = pv_rows(s_d, kvrs[1], 1, k * rq, (k + 1) * rq, tok)
                parts.append(part)
            if k >= 1:
                ofin(_cat1(c_c[(k - 1) * rq:k * rq], parts[k - 1]), NB - 1, (k - 1) * rq, k * rq,
                     wo2[2 * D:])
        while live:
            advance(live[0], 0, None)
        assert not cols

        gb, cb1, sb = mods['gb'], mods['cb1'], mods['sb']
        sel = (S - 1) - (state[0] & 2047)
        sel_idx = [sel[t, 0] for t in range(C)]
        x1s = jnp.concatenate([acc_ref[pl.ds(it, 1), :] for it in sel_idx], axis=0)
        sts = jnp.concatenate([st_ref[pl.ds(it, 1), :] for it in sel_idx], axis=0)
        xn = (x1s - _rep(sts[:, :128])) * _rep(sts[:, 128:])
        xsb = (xn * cb1 + sb).astype(bf16)
        xs = xsb.astype(f32)
        rs = _bf(jnp.sum(xs * wr1, axis=-1, keepdims=True))
        wg = jnp.concatenate([_b16(gu_t[st, 0]) for st in range(NST)], axis=1)
        wu = jnp.concatenate([_b16(gu_t[st, 1]) for st in range(NST)], axis=1)
        g = jnp.dot(xsb, wg, preferred_element_type=f32)
        u = jnp.dot(xsb, wu, preferred_element_type=f32)
        g = _bf(g)
        g = _bf(g * jax.nn.sigmoid(g))
        gu = g * _bf(u)
        nmain = (NST - 1) * 128
        dup = nmain - LAST0
        gu = _cat1(gu[:, :nmain], jnp.where(lane8 >= dup, gu[:, nmain:], 0.0))
        wd = _cat0(_b16(wd_buf[0:nmain // 2, :]), _b16(wd_buf[LAST0 // 2:F // 2, :]))
        y = _bf(jnp.dot(gu.astype(bf16), wd, preferred_element_type=f32))
        y = _bf(y * _bf(jax.nn.sigmoid(rs)))
        newrows = x1s + _bf(gb * _bf(xs + y))

        for i in range(NB):
            out_cp(i).wait()
        sub = lax.broadcasted_iota(i32, (16, M), 0)
        bases = []
        for t in range(C):
            it = sel_idx[t]
            base = pl.multiple_of((it >> 4) << 4, 16)
            bases.append(base)
            cur = out_buf[pl.ds(base, 16), :].astype(f32)
            out_buf[pl.ds(base, 16), :] = jnp.where(sub == (it & 15), newrows[t:t + 1, :], cur).astype(bf16)

        def fix_cp(t):
            return cp(out_buf.at[pl.ds(bases[t], 16), :], out_hbm.at[pl.ds(bases[t], 16), :], SEM_FIX + t)

        uniq = []
        for t in range(C):
            u_ = jnp.bool_(True)
            for t2 in range(t):
                u_ = jnp.logical_and(u_, bases[t] != bases[t2])
            uniq.append(u_)
        for t in range(C):
            pl.when(uniq[t])(lambda t=t: fix_cp(t).start())
        for t in range(C):
            pl.when(uniq[t])(lambda t=t: fix_cp(t).wait())

    prologue()
    lax.fori_loop(0, NP - 2, body, 0)
    final()


@jax.jit
def pallas_adaLN_cond__compressed_kv_cla__moe_arch_mod__prompt_kernel(
    A_x: jax.Array,
    A_c_kv: jax.Array,
    A_w_q: jax.Array,
    A_w_uk: jax.Array,
    A_w_uv: jax.Array,
    A_w_o: jax.Array,
    B_x: jax.Array,
    B_w_r: jax.Array,
    B_w_gate: jax.Array,
    B_w_up: jax.Array,
    B_w_down: jax.Array,
    c: jax.Array,
    w_mod: jax.Array,
):
    x = A_x.reshape(S, M)
    ckv = A_c_kv.reshape(S, DC)
    wo = A_w_o.reshape(H * D, M)
    hbm = pl.BlockSpec(memory_space=pltpu.HBM)

    out = pl.pallas_call(
        _kernel,
        in_specs=[hbm] * 12,
        out_specs=hbm,
        out_shape=jax.ShapeDtypeStruct((S, M), bf16),
        scratch_shapes=[
            pltpu.VMEM((S // 2, M), u32),
            pltpu.VMEM((S // 2, DC), u32),
            pltpu.VMEM((S // 2, M), u32),
            pltpu.VMEM((S, M), f32),
            pltpu.VMEM((2, 2, S // 2, D), u32),
            pltpu.VMEM((2, 2, S // 2, D), u32),
            pltpu.VMEM((S // 2, 2 * D), u32),
            pltpu.VMEM((4, M, D), u32),
            pltpu.VMEM((4, DC, D), u32),
            pltpu.VMEM((4, DC, D), u32),
            pltpu.VMEM((NP * D, M), u32),
            pltpu.VMEM((M // 2, 6 * M), u32),
            pltpu.VMEM((1, M), bf16),
            pltpu.VMEM((M,), bf16),
            pltpu.VMEM((2, F // 2, M), u32),
            pltpu.VMEM((NST, 2, M // 2, 128), u32),
            pltpu.VMEM((F // 2, M), u32),
            pltpu.VMEM((S, M), bf16),
            pltpu.VMEM((HB, HB), i32),
            pltpu.VMEM((S, 256), f32),
            pltpu.SemaphoreType.DMA((NSEM,)),
        ],
        compiler_params=pltpu.CompilerParams(
            vmem_limit_bytes=100 * 1024 * 1024,
            disable_bounds_checks=True,
            disable_semaphore_checks=True,
        ),
    )(x, ckv, A_w_q, A_w_uk, A_w_uv, wo, B_w_r, B_w_gate.T, B_w_up.T, B_w_down, c, w_mod)
    return out.reshape(1, S, M)
```

```python
import jax
import jax.numpy as jnp
from jax import lax
import jax.experimental.pallas as pl
import jax.experimental.pallas.tpu as pltpu

S = 2048
M = 640
DC = 512
H = 32
D = 128
F = 1728
C = 8
TQ = 256
HB = TQ // 2
NB = S // TQ
NP = H // 2
PR = 16
EPS = 1e-5
LOG2E = 1.4426950408889634
NEG = -1e30
QSCALE = (D ** -0.5) * LOG2E
f32 = jnp.float32
bf16 = jnp.bfloat16
u32 = jnp.uint32
i32 = jnp.int32
NT = (((1,), (1,)), ((), ()))

SEM_WQ = 0
SEM_WV = 4
SEM_WO = 8
SEM_GU = 10
SEM_CKV = 14
SEM_X = 18
SEM_C = 20
SEM_MODA = 21
SEM_MODB = 22
SEM_WR = 23
SEM_WD = 24
SEM_OUT = 25
SEM_FIX = 33
SEM_WK = 41
NSEM = 45

NST = 14
LAST0 = F - 128
CKV_CHUNKS = ((0, 1), (1, 3), (3, 6), (6, 8))
X_CHUNKS = ((5, 8), (0, 5))
KT = (2, 3)
S_CHUNK = 3
PAD_ROWS = 400


def _bf(x):
    return x.astype(bf16).astype(f32)


def _unpack_pair(w32):
    lo = pltpu.bitcast(w32 << 16, f32).astype(bf16)
    hi = pltpu.bitcast(w32 & jnp.uint32(0xFFFF0000), f32).astype(bf16)
    return lo, hi


def _b16(x32):
    return pltpu.bitcast(x32, bf16)


def _p32(x16):
    return pltpu.bitcast(x16, u32)


def _tiles(x):
    return [x[:, t * 128:(t + 1) * 128] for t in range(x.shape[1] // 128)]


def _cat0(*xs):
    return jnp.concatenate(xs, axis=0)


def _cat1(*xs):
    return jnp.concatenate(xs, axis=1)


def _bc(v):
    return jnp.broadcast_to(v, (v.shape[0], 128))


def _rep(v):
    return jnp.concatenate([v] * (M // 128), axis=1)


def _bits(v):
    x32 = pltpu.bitcast(v, u32)
    dep = None
    for g in range(x32.shape[0] // 8):
        for t in _tiles(x32[8 * g:8 * g + 8]):
            dep = t if dep is None else dep | t
    return dep


def _anchor(x16, deps):
    if not deps:
        return x16
    x32 = _p32(x16)
    parts = []
    for g in range(x32.shape[0] // 8):
        r = x32[8 * g:8 * g + 8]
        if g in deps:
            t = r[:, :128]
            t = t & (t | deps[g])
            r = t if r.shape[1] == 128 else _cat1(t, r[:, 128:])
        parts.append(r)
    return _b16(jnp.concatenate(parts, axis=0))


def _gate(x, tok):
    if tok is None:
        return x
    t = pltpu.bitcast(x[:, :128], u32)
    t = t & (t | jnp.concatenate([tok] * (x.shape[0] // 8), axis=0))
    t = pltpu.bitcast(t, x.dtype)
    return t if x.shape[1] == 128 else _cat1(t, x[:, 128:])


def _normalize(o, lrun):
    l = jnp.sum(lrun, axis=-1, keepdims=True)
    rc = pl.reciprocal(l, approx=True)
    rc = rc * (2.0 - l * rc)
    return (o * rc).astype(bf16)


def _kernel(x_hbm, ckv_hbm, wq_hbm, wuk_hbm, wuv_hbm, wo_hbm, wr_hbm, wg_hbm, wu_hbm,
            wd_hbm, c_hbm, wmod_hbm, out_hbm,
            x_buf, ckv_buf, h1_ref, acc_ref, k_ref, v_ref, q_ref,
            wq_buf, wk_buf, wv_buf, wo_buf, wmod_buf, c_buf, wr_buf, gu_buf, gu_t, wd_buf,
            out_buf, eye_ref, st_ref, kt_ref, sct_ref, mod_ref, sems):

    def cp(src, dst, s):
        return pltpu.make_async_copy(src, dst, sems.at[s])

    def wq_cp(jj):
        sl = jj & 3
        return cp(wq_hbm.bitcast(u32).at[:, jj, :], wq_buf.at[sl], SEM_WQ + sl)

    def wkv_cp(jj):
        sl = jj & 3
        return [cp(wuk_hbm.bitcast(u32).at[:, jj, :], wk_buf.at[sl], SEM_WK + sl),
                cp(wuv_hbm.bitcast(u32).at[:, jj, :], wv_buf.at[sl], SEM_WV + sl)]

    def wo_cp(part):
        r0, r1 = (0, D) if part == 0 else (D, NP * D)
        return cp(wo_hbm.bitcast(u32).at[r0:r1, :], wo_buf.at[r0:r1, :], SEM_WO + part)

    def ckv_cp(t):
        a, b = CKV_CHUNKS[t]
        return cp(ckv_hbm.bitcast(u32).at[a * HB:b * HB, :], ckv_buf.at[a * HB:b * HB, :], SEM_CKV + t)

    def x_cp(t):
        a, b = X_CHUNKS[t]
        return cp(x_hbm.bitcast(u32).at[a * HB:b * HB, :], x_buf.at[a * HB:b * HB, :], SEM_X + t)

    def c_cp():
        return cp(c_hbm, c_buf, SEM_C)

    def moda_cp():
        return cp(wmod_hbm.bitcast(u32).at[:, 0:2 * M], wmod_buf.at[:, 0:2 * M], SEM_MODA)

    def modb_cp():
        return cp(wmod_hbm.bitcast(u32).at[:, 2 * M:6 * M], wmod_buf.at[:, 2 * M:6 * M], SEM_MODB)

    def late_cps():
        return [cp(wr_hbm, wr_buf, SEM_WR),
                cp(wd_hbm.bitcast(u32), wd_buf, SEM_WD)]

    def gu_cp(part):
        r0, r1 = (0, 64) if part == 0 else (64, F // 2)
        return [cp(w.bitcast(u32).at[r0:r1, :], gu_buf.at[n, r0:r1, :], SEM_GU + 2 * part + n)
                for n, w in enumerate((wg_hbm, wu_hbm))]

    def out_cp(i):
        return cp(out_buf.at[i * TQ:(i + 1) * TQ, :], out_hbm.at[i * TQ:(i + 1) * TQ, :], SEM_OUT + i)

    def silu_c():
        c = c_buf[...].astype(f32)
        sc = (c * jax.nn.sigmoid(c)).astype(bf16)
        return jnp.broadcast_to(sc, (8, M))

    def get_wq(jj):
        return jnp.concatenate(_unpack_pair(wq_buf[jj & 3]), axis=1)

    def get_wkv(jj):
        return jnp.concatenate(_unpack_pair(wk_buf[jj & 3]) + _unpack_pair(wv_buf[jj & 3]), axis=1)

    def get_wo(jj):
        st = jj * D if isinstance(jj, int) else pl.multiple_of(jj * D, D)
        return _b16(wo_buf[pl.ds(st, D), :])

    def kv_refs(jj):
        sl = jj & 1
        return k_ref.at[sl], v_ref.at[sl], kt_ref.at[sl]

    def rows(i):
        return slice(i * TQ, (i + 1) * TQ)

    def hrows(i):
        return slice(i * HB, (i + 1) * HB)

    clock = [0]
    hooks = {'take': None, 'post': None}

    def post(res, dur):
        if hooks['post']:
            hooks['post'](res, dur)

    def take(ng):
        return hooks['take'](ng) if hooks['take'] else {}

    def qproj(wq, i, r0=0, r1=TQ):
        h = _b16(h1_ref[i * HB + r0 // 2:i * HB + r1 // 2, :])
        q = jnp.dot(h, wq, preferred_element_type=f32)
        clock[0] += (r1 - r0) * 5 * (wq.shape[1] // D) // 4
        return (q * QSCALE).astype(bf16)

    def qstore(wq, i, r0=0, r1=TQ):
        q_ref[i * HB + r0 // 2:i * HB + r1 // 2, :] = _p32(qproj(wq, i, r0, r1))

    def qload(i):
        return _b16(q_ref[hrows(i), :])

    def kvproj(wkv, kvr, i):
        kr, vr = kvr[:2]
        kv = _tiles(jnp.dot(_b16(ckv_buf[hrows(i), :]), wkv, preferred_element_type=f32))
        for hh in range(2):
            k32 = _p32(kv[hh].astype(bf16))
            kr[hh, hrows(i), :] = k32
            if hh == 0 and i in KT:
                kvr[2][i - KT[0]] = _p32(_b16(k32).T)
            vr[hh, hrows(i), :] = _p32(kv[2 + hh].astype(bf16))

    row = lax.broadcasted_iota(i32, (HB, HB), 0)
    col = lax.broadcasted_iota(i32, (HB, HB), 1)

    def scores(q, kvr, hh, i, lead=False):
        kr = kvr[0]
        tri = col <= row
        qb = q[:, hh * D:(hh + 1) * D]
        nt = 2 * i + 1
        tiles = {}
        mrun = None
        todo = list(range(nt))
        if lead:
            kt = _cat1(_b16(kvr[2][0]), _b16(kvr[2][1]))
            for t, v in enumerate(_tiles(jnp.dot(qb, kt, preferred_element_type=f32))):
                tiles[2 * KT[0] + t] = v
                mrun = v if mrun is None else jnp.maximum(mrun, v)
            todo = [t for t in todo if t not in tiles]
        groups = []
        for t in todo:
            if groups and len(groups[-1]) < S_CHUNK and groups[-1][-1] == t - 1:
                groups[-1].append(t)
            else:
                groups.append([t])
        for grp in groups:
            c0, c1 = grp[0], grp[-1] + 1
            sc = lax.dot_general(_anchor(qb, take(4 * (c1 - c0))), _b16(kr[hh, c0 * 64:c1 * 64, :]), NT,
                                 preferred_element_type=f32)
            post(sc, 64 * (c1 - c0))
            clock[0] += 64 * (c1 - c0)
            ts = _tiles(sc)
            if c1 == nt:
                last = ts[-1]
                ts[-1] = _cat0(jnp.where(tri, last[:HB], NEG), last[HB:])
            for t, v in enumerate(ts):
                mrun = v if mrun is None else jnp.maximum(mrun, v)
                tiles[c0 + t] = v
        tiles = [tiles[t] for t in range(nt)]
        s_ext = lax.dot_general(qb[HB:], _b16(kr[hh, nt * 64:(nt + 1) * 64, :]), NT,
                                preferred_element_type=f32)
        clock[0] += 32
        s_ext = jnp.where(tri, s_ext, NEG)
        mrun = _cat0(mrun[:HB], jnp.maximum(mrun[HB:], s_ext))
        m = jnp.max(mrun, axis=-1, keepdims=True)
        return tiles, s_ext, m

    def pv(s, kvr, hh, chunk=2, tie=False):
        vr = kvr[1]
        tiles, s_ext, m = s
        mb = jnp.broadcast_to(m, (TQ, 128))
        lrun = None
        o = None
        for c0 in range(0, len(tiles), chunk):
            ps = [jnp.exp2(t - mb) for t in tiles[c0:c0 + chunk]]
            for p in ps:
                lrun = p if lrun is None else lrun + p
            if tie and lrun is not ps[-1]:
                ps[-1] = jnp.minimum(ps[-1], lrun)
            pc = jnp.concatenate(ps, axis=1).astype(bf16)
            pc = _anchor(pc, take(4 * len(ps)))
            oc = jnp.dot(pc, _b16(vr[hh, c0 * 64:(c0 + len(ps)) * 64, :]), preferred_element_type=f32)
            o = oc if o is None else o + oc
            clock[0] += 64 * len(ps)
        nt = len(tiles)
        p_ext = jnp.exp2(s_ext - mb[HB:])
        o_ext = jnp.dot(p_ext.astype(bf16), _b16(vr[hh, nt * 64:(nt + 1) * 64, :]),
                        preferred_element_type=f32)
        post(o_ext, 128)
        clock[0] += 32
        lrun = _cat0(lrun[:HB], lrun[HB:] + p_ext)
        o = _cat0(o[:HB], o[HB:] + o_ext)
        return _normalize(o, lrun)

    def pv_rows(s, kvr, hh, r0, r1, rel):
        vr = kvr[1]
        tiles, s_ext, m = s
        ts_all = [t[r0:r1] for t in tiles]
        if r0 >= HB:
            ts_all.append(s_ext[r0 - HB:r1 - HB])
        mb = _gate(jnp.broadcast_to(m[r0:r1], (r1 - r0, 128)), rel)
        lrun = None
        o = None
        tok = None
        for c0 in range(0, len(ts_all), 4):
            ps = [jnp.exp2(t - mb) for t in ts_all[c0:c0 + 4]]
            for p in ps:
                lrun = p if lrun is None else lrun + p
            pc = jnp.concatenate(ps, axis=1).astype(bf16)
            oc = jnp.dot(pc, _b16(vr[hh, c0 * 64:(c0 + len(ps)) * 64, :]), preferred_element_type=f32)
            o = oc if o is None else o + oc
            if c0 == 0:
                tok = pltpu.bitcast(oc[0:8], u32)
        return _normalize(o, lrun), tok

    def prologue():
        first = ([ckv_cp(0)] + wkv_cp(0) + [ckv_cp(t) for t in range(1, 4)] + wkv_cp(1)
                 + [c_cp(), moda_cp(), x_cp(0), wq_cp(0), x_cp(1), wq_cp(1), wo_cp(0)]
                 + gu_cp(0) + wkv_cp(2) + [wq_cp(2)] + wkv_cp(3) + [wo_cp(1)] + gu_cp(1) + [modb_cp()] + late_cps())
        for c_ in first:
            c_.start()
        acc_ref[...] = jnp.zeros_like(acc_ref)
        eye_ref[...] = jnp.where(col == row, -1, 0).astype(i32)
        h1_ref[0:PAD_ROWS, :] = jnp.zeros((PAD_ROWS, M), u32)

        for c_ in wkv_cp(0):
            c_.wait()
        ckv_cp(0).wait()
        wkv = get_wkv(0)
        kvr = kv_refs(0)
        kvproj(wkv, kvr, 0)
        ckv_cp(1).wait()
        kvproj(wkv, kvr, 1)
        kvproj(wkv, kvr, 2)
        ckv_cp(2).wait()
        for i in range(3, 6):
            kvproj(wkv, kvr, i)
        ckv_cp(3).wait()
        for c_ in wkv_cp(1):
            c_.wait()
        kvproj(wkv, kvr, 6)
        kvproj(wkv, kvr, 7)
        wkv = get_wkv(1)
        kvr = kv_refs(1)
        for i in range(5):
            kvproj(wkv, kvr, i)
        c_cp().wait()
        moda_cp().wait()
        x_cp(0).wait()
        wq_cp(0).wait()
        mod = _bf(jnp.dot(silu_c(), _b16(wmod_buf[:, 0:2 * M]), preferred_element_type=f32))
        sct_ref[...] = jnp.broadcast_to(silu_c()[0:1].astype(f32), (128, M)).T
        sa = mod[0:1, 0:M]
        ca1 = 1.0 + mod[0:1, M:2 * M]
        wq = get_wq(0)

        def ln1q(i, split=False):
            for r0 in range(i * TQ, (i + 1) * TQ, PR):
                x = _b16(x_buf[r0 // 2:(r0 + PR) // 2, :]).astype(f32)
                xc = x - _rep(_bc(jnp.sum(x, axis=-1, keepdims=True)) * (1.0 / M))
                sv = _bc(jnp.sum(xc * xc, axis=-1, keepdims=True))
                rstd = lax.rsqrt(sv * (1.0 / M) + EPS)
                h1_ref[r0 // 2:(r0 + PR) // 2, :] = _p32((xc * _rep(rstd) * ca1 + sa).astype(bf16))
            for r0, r1 in (((0, HB), (HB, TQ)) if split else ((0, TQ),)):
                qstore(wq, i, r0, r1)

        kvproj(wkv, kvr, 5)
        ln1q(7)
        ln1q(6)
        ln1q(5, True)
        x_cp(1).wait()
        kvproj(wkv, kvr, 6)
        ln1q(4)
        kvproj(wkv, kvr, 7)
        ln1q(3)
        ln1q(2)
        ln1q(1)
        ln1q(0, True)
        wq_cp(1).wait()
        wo_cp(0).wait()
        for c_ in wkv_cp(2) + gu_cp(0):
            c_.wait()

    def body(j, carry):
        @pl.when(j + 3 < NP)
        def _():
            wq_cp(j + 3).start()

        @pl.when(j + 4 < NP)
        def _():
            for c_ in wkv_cp(j + 4):
                c_.start()

        wq_n = get_wq(j + 1)
        wkv_n = get_wkv(j + 2)
        kvr = kv_refs(j)

        def oproj(ctx, i):
            acc_ref[rows(i), :] += jnp.dot(ctx, get_wo(j), preferred_element_type=f32)

        def kvhalf(i, n):
            kv = _tiles(jnp.dot(_b16(ckv_buf[hrows(i), :]), wkv_n[:, n * 2 * D:(n + 1) * 2 * D],
                                preferred_element_type=f32))
            for hh in range(2):
                k32 = _p32(kv[hh].astype(bf16))
                kvr[n][hh, hrows(i), :] = k32
                if n == 0 and hh == 0 and i in KT:
                    kvr[2][i - KT[0]] = _p32(_b16(k32).T)

        qs = {}

        def qnext(i):
            if i >= 0:
                if i not in qs:
                    qs[i] = qload(i)
                qstore(wq_n, i)

        qs[NB - 1] = qload(NB - 1)
        prev = None
        for i in range(NB - 1, -1, -1):
            top = i == NB - 1
            s_a = scores(qs[i], kvr, 0, i, top)
            if top:
                qnext(i)
            else:
                qnext(i - 1)
                kvhalf(i + 1, 0)
            c_a = pv(s_a, kvr, 0, 2, True)
            s_b = scores(qs[i], kvr, 1, i)
            if top:
                qnext(i - 1)
            else:
                kvhalf(i + 1, 1)
                oproj(prev, i + 1)
            c_b = pv(s_b, kvr, 1, 3 if top else 2, True)
            prev = _cat1(c_a, c_b)
        kvproj(wkv_n, kvr, 0)
        oproj(prev, 0)
        for n in range(2):
            r0 = pl.multiple_of(jnp.minimum(j * 64, LAST0 // 2), 32)
            gu_t[j, n] = _p32(_b16(gu_buf[n, pl.ds(r0, 64), :]).T)

        nm = jnp.clip(j - 2, 0, 9)
        c0 = pl.multiple_of(jnp.where(j >= 2, 2 * M + 256 * nm, 0), 256)
        wm = _b16(wmod_buf[:, pl.ds(c0, 256)]).astype(f32)
        sct = sct_ref[...]
        pm = wm * _cat1(sct, sct)
        am = pm[0:8]
        for g in range(1, M // 8):
            am = am + pm[8 * g:8 * g + 8]
        mod_ref[jnp.where(j >= 2, nm, 10)] = am

        wq_cp(j + 2).wait()

        @pl.when(j == 1)
        def _():
            modb_cp().wait()

        @pl.when(j == 0)
        def _():
            for c_ in [wo_cp(1)] + gu_cp(1):
                c_.wait()

        @pl.when(j + 3 < NP)
        def _():
            for c_ in wkv_cp(j + 3):
                c_.wait()
        return carry

    def final():
        ja, jb = NP - 2, NP - 1
        for c_ in late_cps():
            c_.wait()
        wq15 = get_wq(jb)
        kvrs = (kv_refs(ja), kv_refs(jb))
        wo2 = _cat0(get_wo(ja), get_wo(jb))
        mods = {}
        wr1 = wr_buf[...].astype(f32).reshape(1, M)
        sub8 = lax.broadcasted_iota(i32, (8, 128), 0)
        lane8 = lax.broadcasted_iota(i32, (8, 128), 1)
        mod = _bf(jnp.sum(jnp.concatenate([mod_ref[n] for n in range(10)], axis=1), axis=0, keepdims=True))
        mods['ga'] = mod[:, 0:M]
        mods['sb'] = mod[:, M:2 * M]
        mods['cb1'] = _bf(1.0 + mod[:, 2 * M:3 * M])
        mods['gb'] = mod[:, 3 * M:4 * M]
        mods['gc'] = mods['gb'] * mods['cb1']
        mods['gs'] = mods['gb'] * mods['sb']
        mods['wc'] = wr1 * mods['cb1']
        mods['r0'] = jnp.sum(wr1 * mods['sb'], axis=-1, keepdims=True)

        cols = []
        state = [(-(2 ** 27)) + sub8]
        done_rows = {}

        def subsum(v, op):
            for sh in (4, 2, 1):
                v = op(v, pltpu.roll(v, sh, 0))
            return v

        def tree(vs, op):
            while len(vs) > 1:
                vs = [op(vs[k], vs[k + 1]) if k + 1 < len(vs) else vs[k] for k in range(0, len(vs), 2)]
            return vs[0]

        def merge(pend):
            kc = jnp.concatenate(pend, axis=0)
            st = state[0]
            gs = [kc[8 * g:8 * g + 8] for g in range(16)]
            r1 = subsum(tree([kg & eye_ref[8 * g:8 * g + 8, :] for g, kg in enumerate(gs)], jnp.bitwise_or),
                        jnp.bitwise_or)
            r2 = jnp.where(lane8 < 8, subsum(st & eye_ref[0:8, :], jnp.bitwise_or), -(2 ** 28))
            hi = 0.0
            lo = 0.0
            for rr in (r1, r2):
                cnt = tree([(rr - kg) >> 31 for kg in gs + [st]], jnp.add)
                sel = subsum(cnt, jnp.add) + sub8 == 0
                hi = hi + jnp.where(sel, (rr >> 11).astype(f32), 0.0)
                lo = lo + jnp.where(sel, (rr & 2047).astype(f32), 0.0)
            hi = _bc(jnp.sum(hi, axis=-1, keepdims=True)).astype(i32)
            lo = _bc(jnp.sum(lo, axis=-1, keepdims=True)).astype(i32)
            state[0] = (hi << 11) | lo
            return pltpu.bitcast(state[0], u32)

        deferred = []

        def emit_out(r0, x1, xc, rstd):
            of = x1 + (xc * _rep(rstd)) * mods['gc'] + mods['gs']
            out_buf[r0:r0 + PR, :] = of.astype(bf16)
            blk = r0 // TQ
            done_rows[blk] = done_rows.get(blk, 0) + PR
            if done_rows[blk] == TQ:
                out_cp(blk).start()
            return of

        def piece(r0):
            rel = yield
            x1 = acc_ref[r0:r0 + PR, :]
            sm = _bc(jnp.sum(_gate(x1, rel), axis=-1, keepdims=True))
            rel = yield
            m = _gate(sm, rel) * (1.0 / M)
            xc = x1 - _rep(m)
            sv = _bc(jnp.sum(xc * xc, axis=-1, keepdims=True))
            rw = _bc(jnp.sum(xc * mods['wc'], axis=-1, keepdims=True))
            rel = yield
            rstd = lax.rsqrt(_gate(sv, rel) * (1.0 / M) + EPS)
            st_ref[r0:r0 + PR, :] = _cat1(m, rstd)
            if r0 < S - TQ:
                dep = _bits(emit_out(r0, x1, xc, rstd))
            else:
                deferred.append((r0, m, rstd))
                dep = None
            r = _bf(rw * rstd + mods['r0'])
            rb = pltpu.bitcast(r, i32) >> 16
            rb = rb ^ ((rb >> 31) & 0x7FFF)
            idx = (S - 1 - r0) - lax.broadcasted_iota(i32, (PR, 128), 0)
            key = (rb << 11) | idx
            cols.append(key)
            return _bits(key) if dep is None else dep | _bits(key)

        def merge_task(pend):
            rel = yield
            return merge([_gate(pend[0], rel)] + pend[1:])

        live = []
        anchors = []
        nxt = [0]
        stage_gap = 200
        stage_cost = (48, 32, 48, 128)

        def advance(ent, t, rel):
            try:
                ent[2].send(rel)
                ent[0] = t + stage_gap
                ent[1] += 1
            except StopIteration as e:
                anchors.append([t + (530 if ent[1] == 3 else 280), e.value])
                live.remove(ent)
                if len(cols) * PR == 128:
                    g = merge_task(list(cols))
                    del cols[:]
                    next(g)
                    live.insert(0, [t + stage_gap, 3, g])

        def post_impl(res, dur):
            for g in range(min(res.shape[0] // 16, dur // 16)):
                t = clock[0] + 16 * g
                if t < nxt[0]:
                    continue
                for ent in live:
                    if ent[0] <= t:
                        nxt[0] = t + stage_cost[ent[1]]
                        advance(ent, t, pltpu.bitcast(res[16 * g:16 * g + 8, 0:128], u32))
                        break

        def take_impl(ng):
            deps = {}
            for g in range(ng):
                t = clock[0] + 16 * g
                ready = [an for an in anchors if an[0] <= t]
                anchors[:] = [an for an in anchors if an[0] > t]
                for an in ready:
                    deps[g] = an[1] | deps[g] if g in deps else an[1]
            return deps

        def ofin(ctx, i, r0, r1, w):
            rs = slice(i * TQ + r0, i * TQ + r1)
            lhs = _anchor(ctx, take((r1 - r0) // 16))
            a = acc_ref[rs, :] + jnp.dot(lhs, w, preferred_element_type=f32)
            clock[0] += 5 * (r1 - r0) * w.shape[0] // 512
            x = _b16(x_buf[(i * TQ + r0) // 2:(i * TQ + r1) // 2, :]).astype(f32)
            acc_ref[rs, :] = x + mods['ga'] * a
            for r in range(i * TQ + r0, i * TQ + r1, PR):
                g = piece(r)
                next(g)
                live.append([clock[0], 0, g])

        def opart(ctx, i, r0, r1):
            rs = slice(i * TQ + r0, i * TQ + r1)
            lhs = _anchor(ctx[r0:r1], take((r1 - r0) // 16))
            acc_ref[rs, :] += jnp.dot(lhs, wo2[:2 * D], preferred_element_type=f32)
            clock[0] += 5 * (r1 - r0) // 2

        hooks.update(take=take_impl, post=post_impl)
        clock[0] = 0
        q15 = {}
        prev = None
        o1, o2, qs = 80, 192, 64
        for i in range(NB):
            q14 = qload(i)
            lastb = i == NB - 1
            oprev = lambda r0, r1: ofin(prev[r0:r1], i - 1, r0, r1, wo2)
            if i < 3:
                s_a = scores(q14, kvrs[0], 0, i)
                s_b = scores(q14, kvrs[0], 1, i)
                if i == 0:
                    q15[0] = qproj(wq15, 0)
                else:
                    oprev(0, 192)
                c_a = pv(s_a, kvrs[0], 0)
                c_b = pv(s_b, kvrs[0], 1)
                s_c = scores(q15[i], kvrs[1], 0, i)
                s_d = scores(q15[i], kvrs[1], 1, i)
                if i == 0:
                    q15[1] = qproj(wq15, 1)
                else:
                    oprev(192, TQ)
                    q15[i + 1] = qproj(wq15, i + 1)
                c_c = pv(s_c, kvrs[1], 0)
                c_d = pv(s_d, kvrs[1], 1)
            else:
                s_a = scores(q14, kvrs[0], 0, i)
                oprev(0, o1)
                c_a = pv(s_a, kvrs[0], 0)
                s_b = scores(q14, kvrs[0], 1, i)
                oprev(o1, o2)
                c_b = pv(s_b, kvrs[0], 1)
                s_c = scores(q15[i], kvrs[1], 0, i)
                oprev(o2, TQ)
                if lastb:
                    c_ab = _cat1(c_a, c_b)
                    opart(c_ab, i, 0, qs)
                else:
                    qa = qproj(wq15, i + 1, 0, qs)
                c_c = pv(s_c, kvrs[1], 0)
                s_d = scores(q15[i], kvrs[1], 1, i)
                if lastb:
                    opart(c_ab, i, qs, TQ)
                    break
                q15[i + 1] = _cat0(qa, qproj(wq15, i + 1, qs, TQ))
                c_d = pv(s_d, kvrs[1], 1)
            prev = _cat1(c_a, c_b, c_c, c_d)
        hooks.update(take=None, post=None)
        rq = 64
        parts = []
        tok = None
        for k in range(TQ // rq + 1):
            if k < TQ // rq:
                part, tok = pv_rows(s_d, kvrs[1], 1, k * rq, (k + 1) * rq, tok)
                parts.append(part)
            if k >= 1:
                ofin(_cat1(c_c[(k - 1) * rq:k * rq], parts[k - 1]), NB - 1, (k - 1) * rq, k * rq,
                     wo2[2 * D:])
        while live:
            advance(live[0], 0, None)
        assert not cols

        gb, cb1, sb = mods['gb'], mods['cb1'], mods['sb']
        sel = (S - 1) - (state[0] & 2047)
        sel_idx = [sel[t, 0] for t in range(C)]
        x1s = jnp.concatenate([acc_ref[pl.ds(it, 1), :] for it in sel_idx], axis=0)
        sts = jnp.concatenate([st_ref[pl.ds(it, 1), :] for it in sel_idx], axis=0)
        xn = (x1s - _rep(sts[:, :128])) * _rep(sts[:, 128:])
        xsb = (xn * cb1 + sb).astype(bf16)
        xs = xsb.astype(f32)
        rs = _bf(jnp.sum(xs * wr1, axis=-1, keepdims=True))
        wg = jnp.concatenate([_b16(gu_t[st, 0]) for st in range(NST)], axis=1)
        wu = jnp.concatenate([_b16(gu_t[st, 1]) for st in range(NST)], axis=1)
        g = jnp.dot(xsb, wg, preferred_element_type=f32)
        u = jnp.dot(xsb, wu, preferred_element_type=f32)
        toks = [pltpu.bitcast(t, u32) for t in _tiles(g)]
        for k, (r0, m, rstd) in enumerate(deferred):
            x1 = acc_ref[r0:r0 + PR, :]
            emit_out(r0, x1, x1 - _rep(_gate(m, toks[k // 2])), rstd)
        g = _bf(g)
        g = _bf(g * jax.nn.sigmoid(g))
        gu = g * _bf(u)
        nmain = (NST - 1) * 128
        dup = nmain - LAST0
        gu = _cat1(gu[:, :nmain], jnp.where(lane8 >= dup, gu[:, nmain:], 0.0))
        wd = _cat0(_b16(wd_buf[0:nmain // 2, :]), _b16(wd_buf[LAST0 // 2:F // 2, :]))
        y = _bf(jnp.dot(gu.astype(bf16), wd, preferred_element_type=f32))
        y = _bf(y * _bf(jax.nn.sigmoid(rs)))
        newrows = x1s + _bf(gb * _bf(xs + y))

        for i in range(NB):
            out_cp(i).wait()
        sub = lax.broadcasted_iota(i32, (8, M), 0)
        bases = []
        for t in range(C):
            it = sel_idx[t]
            base = pl.multiple_of((it >> 3) << 3, 8)
            bases.append(base)
            cur = out_buf[pl.ds(base, 8), :].astype(f32)
            out_buf[pl.ds(base, 8), :] = jnp.where(sub == (it & 7), newrows[t:t + 1, :], cur).astype(bf16)

        def fix_cp(t):
            return cp(out_buf.at[pl.ds(bases[t], 8), :], out_hbm.at[pl.ds(bases[t], 8), :], SEM_FIX + t)

        uniq = []
        for t in range(C):
            u_ = jnp.bool_(True)
            for t2 in range(t):
                u_ = jnp.logical_and(u_, bases[t] != bases[t2])
            uniq.append(u_)
        for t in range(C):
            pl.when(uniq[t])(lambda t=t: fix_cp(t).start())
        for t in range(C):
            pl.when(uniq[t])(lambda t=t: fix_cp(t).wait())

    prologue()
    lax.fori_loop(0, NP - 2, body, 0)
    final()


@jax.jit
def pallas_adaLN_cond__compressed_kv_cla__moe_arch_mod__prompt_kernel(
    A_x: jax.Array,
    A_c_kv: jax.Array,
    A_w_q: jax.Array,
    A_w_uk: jax.Array,
    A_w_uv: jax.Array,
    A_w_o: jax.Array,
    B_x: jax.Array,
    B_w_r: jax.Array,
    B_w_gate: jax.Array,
    B_w_up: jax.Array,
    B_w_down: jax.Array,
    c: jax.Array,
    w_mod: jax.Array,
):
    x = A_x.reshape(S, M)
    ckv = A_c_kv.reshape(S, DC)
    wo = A_w_o.reshape(H * D, M)
    hbm = pl.BlockSpec(memory_space=pltpu.HBM)

    out = pl.pallas_call(
        _kernel,
        in_specs=[hbm] * 12,
        out_specs=hbm,
        out_shape=jax.ShapeDtypeStruct((S, M), bf16),
        scratch_shapes=[
            pltpu.VMEM((S // 2, M), u32),
            pltpu.VMEM((S // 2, DC), u32),
            pltpu.VMEM((S // 2, M), u32),
            pltpu.VMEM((S, M), f32),
            pltpu.VMEM((2, 2, S // 2, D), u32),
            pltpu.VMEM((2, 2, S // 2, D), u32),
            pltpu.VMEM((S // 2, 2 * D), u32),
            pltpu.VMEM((4, M, D), u32),
            pltpu.VMEM((4, DC, D), u32),
            pltpu.VMEM((4, DC, D), u32),
            pltpu.VMEM((NP * D, M), u32),
            pltpu.VMEM((M // 2, 6 * M), u32),
            pltpu.VMEM((1, M), bf16),
            pltpu.VMEM((M,), bf16),
            pltpu.VMEM((2, F // 2, M), u32),
            pltpu.VMEM((NST, 2, M // 2, 128), u32),
            pltpu.VMEM((F // 2, M), u32),
            pltpu.VMEM((S, M), bf16),
            pltpu.VMEM((HB, HB), i32),
            pltpu.VMEM((S, 256), f32),
            pltpu.VMEM((2, 2, D // 2, TQ), u32),
            pltpu.VMEM((M, 128), f32),
            pltpu.VMEM((11, 8, 256), f32),
            pltpu.SemaphoreType.DMA((NSEM,)),
        ],
        compiler_params=pltpu.CompilerParams(
            vmem_limit_bytes=100 * 1024 * 1024,
            disable_bounds_checks=True,
            disable_semaphore_checks=True,
        ),
    )(x, ckv, A_w_q, A_w_uk, A_w_uv, wo, B_w_r, B_w_gate.T, B_w_up.T, B_w_down, c, w_mod)
    return out.reshape(1, S, M)
```

```python
import jax
import jax.numpy as jnp
from jax import lax
import jax.experimental.pallas as pl
import jax.experimental.pallas.tpu as pltpu

S = 2048
M = 640
DC = 512
H = 32
D = 128
F = 1728
C = 8
TQ = 256
HB = TQ // 2
NB = S // TQ
NP = H // 2
PR1 = 16
PR = 8
EPS = 1e-5
LOG2E = 1.4426950408889634
NEG = -1e30
QSCALE = (D ** -0.5) * LOG2E
f32 = jnp.float32
bf16 = jnp.bfloat16
u32 = jnp.uint32
i32 = jnp.int32
NT = (((1,), (1,)), ((), ()))

SEM_WQ = 0
SEM_WV = 4
SEM_WO = 8
SEM_GU = 10
SEM_CKV = 14
SEM_X = 18
SEM_C = 20
SEM_MODA = 21
SEM_MODB = 22
SEM_WR = 23
SEM_WD = 24
SEM_OUT = 25
SEM_FIX = 33
SEM_WK = 41
NSEM = 45

NST = 14
LAST0 = F - 128
CKV_CHUNKS = ((0, 1), (1, 3), (3, 6), (6, 8))
X_CHUNKS = ((5, 8), (0, 5))
KT = (1, 2)
PAD_ROWS = 400


def _bf(x):
    return x.astype(bf16).astype(f32)


def _unpack_pair(w32):
    lo = pltpu.bitcast(w32 << 16, f32).astype(bf16)
    hi = pltpu.bitcast(w32 & jnp.uint32(0xFFFF0000), f32).astype(bf16)
    return lo, hi


def _b16(x32):
    return pltpu.bitcast(x32, bf16)


def _p32(x16):
    return pltpu.bitcast(x16, u32)


def _tiles(x):
    return [x[:, t * 128:(t + 1) * 128] for t in range(x.shape[1] // 128)]


def _cat0(*xs):
    return jnp.concatenate(xs, axis=0)


def _cat1(*xs):
    return jnp.concatenate(xs, axis=1)


def _bc(v):
    return jnp.broadcast_to(v, (v.shape[0], 128))


def _rep(v):
    return jnp.concatenate([v] * (M // 128), axis=1)


def _bits(v):
    x32 = pltpu.bitcast(v, u32)
    dep = None
    for g in range(x32.shape[0] // 8):
        for t in _tiles(x32[8 * g:8 * g + 8]):
            dep = t if dep is None else dep | t
    return dep


def _anchor(x16, deps):
    if not deps:
        return x16
    x32 = _p32(x16)
    parts = []
    for g in range(x32.shape[0] // 8):
        r = x32[8 * g:8 * g + 8]
        if g in deps:
            t = r[:, :128]
            t = t & (t | deps[g])
            r = t if r.shape[1] == 128 else _cat1(t, r[:, 128:])
        parts.append(r)
    return _b16(jnp.concatenate(parts, axis=0))


def _gate(x, tok):
    if tok is None:
        return x
    t = pltpu.bitcast(x[:, :128], u32)
    t = t & (t | jnp.concatenate([tok] * (x.shape[0] // 8), axis=0))
    t = pltpu.bitcast(t, x.dtype)
    return t if x.shape[1] == 128 else _cat1(t, x[:, 128:])


def _normalize(o, lrun):
    l = jnp.sum(lrun, axis=-1, keepdims=True)
    rc = pl.reciprocal(l, approx=True)
    rc = rc * (2.0 - l * rc)
    return (o * rc).astype(bf16)


def _kernel(x_hbm, ckv_hbm, wq_hbm, wuk_hbm, wuv_hbm, wo_hbm, wr_hbm, wg_hbm, wu_hbm,
            wd_hbm, c_hbm, wmod_hbm, out_hbm,
            x_buf, ckv_buf, h1_ref, acc_ref, k_ref, v_ref, q_ref,
            wq_buf, wk_buf, wv_buf, wo_buf, wmod_buf, c_buf, wr_buf, gu_buf, gu_t, wd_buf,
            out_buf, eye_ref, st_ref, kt_ref, sct_ref, mod_ref, sems):

    def cp(src, dst, s):
        return pltpu.make_async_copy(src, dst, sems.at[s])

    def wq_cp(jj):
        sl = jj & 3
        return cp(wq_hbm.bitcast(u32).at[:, jj, :], wq_buf.at[sl], SEM_WQ + sl)

    def wkv_cp(jj):
        sl = jj & 3
        return [cp(wuk_hbm.bitcast(u32).at[:, jj, :], wk_buf.at[sl], SEM_WK + sl),
                cp(wuv_hbm.bitcast(u32).at[:, jj, :], wv_buf.at[sl], SEM_WV + sl)]

    def wo_cp(part):
        r0, r1 = (0, D) if part == 0 else (D, NP * D)
        return cp(wo_hbm.bitcast(u32).at[r0:r1, :], wo_buf.at[r0:r1, :], SEM_WO + part)

    def ckv_cp(t):
        a, b = CKV_CHUNKS[t]
        return cp(ckv_hbm.bitcast(u32).at[a * HB:b * HB, :], ckv_buf.at[a * HB:b * HB, :], SEM_CKV + t)

    def x_cp(t):
        a, b = X_CHUNKS[t]
        return cp(x_hbm.bitcast(u32).at[a * HB:b * HB, :], x_buf.at[a * HB:b * HB, :], SEM_X + t)

    def c_cp():
        return cp(c_hbm, c_buf, SEM_C)

    def moda_cp():
        return cp(wmod_hbm.bitcast(u32).at[:, 0:2 * M], wmod_buf.at[:, 0:2 * M], SEM_MODA)

    def modb_cp():
        return cp(wmod_hbm.bitcast(u32).at[:, 2 * M:6 * M], wmod_buf.at[:, 2 * M:6 * M], SEM_MODB)

    def late_cps():
        return [cp(wr_hbm, wr_buf, SEM_WR),
                cp(wd_hbm.bitcast(u32), wd_buf, SEM_WD)]

    def gu_cp(part):
        r0, r1 = (0, 64) if part == 0 else (64, F // 2)
        return [cp(w.bitcast(u32).at[r0:r1, :], gu_buf.at[n, r0:r1, :], SEM_GU + 2 * part + n)
                for n, w in enumerate((wg_hbm, wu_hbm))]

    def out_cp(i):
        return cp(out_buf.at[i * TQ:(i + 1) * TQ, :], out_hbm.at[i * TQ:(i + 1) * TQ, :], SEM_OUT + i)

    def silu_c():
        c = c_buf[...].astype(f32)
        sc = (c * jax.nn.sigmoid(c)).astype(bf16)
        return jnp.broadcast_to(sc, (8, M))

    def get_wq(jj):
        return jnp.concatenate(_unpack_pair(wq_buf[jj & 3]), axis=1)

    def get_wkv(jj):
        return jnp.concatenate(_unpack_pair(wk_buf[jj & 3]) + _unpack_pair(wv_buf[jj & 3]), axis=1)

    def get_wo(jj):
        st = jj * D if isinstance(jj, int) else pl.multiple_of(jj * D, D)
        return _b16(wo_buf[pl.ds(st, D), :])

    def kv_refs(jj):
        sl = jj & 1
        return k_ref.at[sl], v_ref.at[sl], kt_ref.at[sl]

    def rows(i):
        return slice(i * TQ, (i + 1) * TQ)

    def hrows(i):
        return slice(i * HB, (i + 1) * HB)

    clock = [0]
    hooks = {'take': None, 'post': None, 'chunk': 3}

    def post(res, dur):
        if hooks['post']:
            hooks['post'](res, dur)

    def take(ng):
        return hooks['take'](ng) if hooks['take'] else {}

    def qproj(wq, i, r0=0, r1=TQ):
        h = _b16(h1_ref[i * HB + r0 // 2:i * HB + r1 // 2, :])
        q = jnp.dot(h, wq, preferred_element_type=f32)
        clock[0] += (r1 - r0) * 5 * (wq.shape[1] // D) // 4
        return (q * QSCALE).astype(bf16)

    def qstore(wq, i, r0=0, r1=TQ):
        q_ref[i * HB + r0 // 2:i * HB + r1 // 2, :] = _p32(qproj(wq, i, r0, r1))

    def qload(i):
        return _b16(q_ref[hrows(i), :])

    def kvproj(wkv, kvr, i):
        kr, vr = kvr[:2]
        kv = _tiles(jnp.dot(_b16(ckv_buf[hrows(i), :]), wkv, preferred_element_type=f32))
        for hh in range(2):
            k32 = _p32(kv[hh].astype(bf16))
            kr[hh, hrows(i), :] = k32
            if hh == 0 and i in KT:
                kvr[2][i - KT[0]] = _p32(_b16(k32).T)
            vr[hh, hrows(i), :] = _p32(kv[2 + hh].astype(bf16))

    row = lax.broadcasted_iota(i32, (HB, HB), 0)
    col = lax.broadcasted_iota(i32, (HB, HB), 1)

    def scores(q, kvr, hh, i, lead=False):
        kr = kvr[0]
        tri = col <= row
        qb = q[:, hh * D:(hh + 1) * D]
        nt = 2 * i + 1
        tiles = {}
        mrun = None
        todo = list(range(nt))
        if lead:
            kt = _cat1(_b16(kvr[2][0]), _b16(kvr[2][1]))
            for t, v in enumerate(_tiles(jnp.dot(qb, kt, preferred_element_type=f32))):
                tiles[2 * KT[0] + t] = v
                mrun = v if mrun is None else jnp.maximum(mrun, v)
            todo = [t for t in todo if t not in tiles]
        groups = []
        for t in todo:
            if groups and len(groups[-1]) < hooks['chunk'] and groups[-1][-1] == t - 1:
                groups[-1].append(t)
            else:
                groups.append([t])
        for grp in groups:
            c0, c1 = grp[0], grp[-1] + 1
            sc = lax.dot_general(_anchor(qb, take(4 * (c1 - c0))), _b16(kr[hh, c0 * 64:c1 * 64, :]), NT,
                                 preferred_element_type=f32)
            post(sc, 64 * (c1 - c0))
            clock[0] += 64 * (c1 - c0)
            ts = _tiles(sc)
            if c1 == nt:
                last = ts[-1]
                ts[-1] = _cat0(jnp.where(tri, last[:HB], NEG), last[HB:])
            for t, v in enumerate(ts):
                mrun = v if mrun is None else jnp.maximum(mrun, v)
                tiles[c0 + t] = v
        tiles = [tiles[t] for t in range(nt)]
        s_ext = lax.dot_general(qb[HB:], _b16(kr[hh, nt * 64:(nt + 1) * 64, :]), NT,
                                preferred_element_type=f32)
        clock[0] += 32
        s_ext = jnp.where(tri, s_ext, NEG)
        mrun = _cat0(mrun[:HB], jnp.maximum(mrun[HB:], s_ext))
        m = jnp.max(mrun, axis=-1, keepdims=True)
        return tiles, s_ext, m

    def pv(s, kvr, hh, chunk=2, tie=False):
        vr = kvr[1]
        tiles, s_ext, m = s
        mb = jnp.broadcast_to(m, (TQ, 128))
        lrun = None
        o = None
        for c0 in range(0, len(tiles), chunk):
            ps = [jnp.exp2(t - mb) for t in tiles[c0:c0 + chunk]]
            for p in ps:
                lrun = p if lrun is None else lrun + p
            if tie and lrun is not ps[-1]:
                ps[-1] = jnp.minimum(ps[-1], lrun)
            pc = jnp.concatenate(ps, axis=1).astype(bf16)
            pc = _anchor(pc, take(4 * len(ps)))
            oc = jnp.dot(pc, _b16(vr[hh, c0 * 64:(c0 + len(ps)) * 64, :]), preferred_element_type=f32)
            o = oc if o is None else o + oc
            clock[0] += 64 * len(ps)
        nt = len(tiles)
        p_ext = jnp.exp2(s_ext - mb[HB:])
        o_ext = jnp.dot(p_ext.astype(bf16), _b16(vr[hh, nt * 64:(nt + 1) * 64, :]),
                        preferred_element_type=f32)
        post(o_ext, 128)
        clock[0] += 32
        lrun = _cat0(lrun[:HB], lrun[HB:] + p_ext)
        o = _cat0(o[:HB], o[HB:] + o_ext)
        return _normalize(o, lrun)

    def pv_rows(s, kvr, hh, r0, r1, rel):
        vr = kvr[1]
        tiles, s_ext, m = s
        ts_all = [t[r0:r1] for t in tiles]
        if r0 >= HB:
            ts_all.append(s_ext[r0 - HB:r1 - HB])
        mb = _gate(jnp.broadcast_to(m[r0:r1], (r1 - r0, 128)), rel)
        lrun = None
        o = None
        tok = None
        for c0 in range(0, len(ts_all), 4):
            ps = [jnp.exp2(t - mb) for t in ts_all[c0:c0 + 4]]
            for p in ps:
                lrun = p if lrun is None else lrun + p
            pc = jnp.concatenate(ps, axis=1).astype(bf16)
            oc = jnp.dot(pc, _b16(vr[hh, c0 * 64:(c0 + len(ps)) * 64, :]), preferred_element_type=f32)
            o = oc if o is None else o + oc
            if c0 == 0:
                tok = pltpu.bitcast(oc[0:8], u32)
        return _normalize(o, lrun), tok

    def prologue():
        first = ([ckv_cp(0)] + wkv_cp(0) + [ckv_cp(t) for t in range(1, 4)] + wkv_cp(1)
                 + [c_cp(), moda_cp(), x_cp(0), wq_cp(0), x_cp(1), wq_cp(1), wo_cp(0)]
                 + gu_cp(0) + wkv_cp(2) + [wq_cp(2)] + wkv_cp(3) + [wo_cp(1)] + gu_cp(1) + [modb_cp()] + late_cps())
        for c_ in first:
            c_.start()
        acc_ref[...] = jnp.zeros_like(acc_ref)
        eye_ref[...] = jnp.where(col == row, -1, 0).astype(i32)
        h1_ref[0:PAD_ROWS, :] = jnp.zeros((PAD_ROWS, M), u32)

        for c_ in wkv_cp(0):
            c_.wait()
        ckv_cp(0).wait()
        wkv = get_wkv(0)
        kvr = kv_refs(0)
        kvproj(wkv, kvr, 0)
        ckv_cp(1).wait()
        kvproj(wkv, kvr, 1)
        kvproj(wkv, kvr, 2)
        ckv_cp(2).wait()
        for i in range(3, 6):
            kvproj(wkv, kvr, i)
        ckv_cp(3).wait()
        for c_ in wkv_cp(1):
            c_.wait()
        kvproj(wkv, kvr, 6)
        kvproj(wkv, kvr, 7)
        wkv = get_wkv(1)
        kvr = kv_refs(1)
        for i in range(5):
            kvproj(wkv, kvr, i)
        c_cp().wait()
        moda_cp().wait()
        x_cp(0).wait()
        wq_cp(0).wait()
        mod = _bf(jnp.dot(silu_c(), _b16(wmod_buf[:, 0:2 * M]), preferred_element_type=f32))
        sct_ref[...] = jnp.broadcast_to(silu_c()[0:1].astype(f32), (128, M)).T
        sa = mod[0:1, 0:M]
        ca1 = 1.0 + mod[0:1, M:2 * M]
        wq = get_wq(0)

        def ln1q(i, split=False):
            for r0 in range(i * TQ, (i + 1) * TQ, PR1):
                x = _b16(x_buf[r0 // 2:(r0 + PR1) // 2, :]).astype(f32)
                xc = x - _rep(_bc(jnp.sum(x, axis=-1, keepdims=True)) * (1.0 / M))
                sv = _bc(jnp.sum(xc * xc, axis=-1, keepdims=True))
                rstd = lax.rsqrt(sv * (1.0 / M) + EPS)
                h1_ref[r0 // 2:(r0 + PR1) // 2, :] = _p32((xc * _rep(rstd) * ca1 + sa).astype(bf16))
            for r0, r1 in (((0, HB), (HB, TQ)) if split else ((0, TQ),)):
                qstore(wq, i, r0, r1)

        kvproj(wkv, kvr, 5)
        ln1q(7)
        ln1q(6)
        ln1q(5, True)
        x_cp(1).wait()
        kvproj(wkv, kvr, 6)
        ln1q(4)
        kvproj(wkv, kvr, 7)
        ln1q(3)
        ln1q(2)
        ln1q(1)
        ln1q(0, True)
        wq_cp(1).wait()
        wo_cp(0).wait()
        for c_ in wkv_cp(2) + gu_cp(0):
            c_.wait()

    def body(j, carry):
        @pl.when(j + 3 < NP)
        def _():
            wq_cp(j + 3).start()

        @pl.when(j + 4 < NP)
        def _():
            for c_ in wkv_cp(j + 4):
                c_.start()

        wq_n = get_wq(j + 1)
        wkv_n = get_wkv(j + 2)
        kvr = kv_refs(j)

        def oproj(ctx, i):
            acc_ref[rows(i), :] += jnp.dot(ctx, get_wo(j), preferred_element_type=f32)

        def kvhalf(i, n):
            kv = _tiles(jnp.dot(_b16(ckv_buf[hrows(i), :]), wkv_n[:, n * 2 * D:(n + 1) * 2 * D],
                                preferred_element_type=f32))
            for hh in range(2):
                k32 = _p32(kv[hh].astype(bf16))
                kvr[n][hh, hrows(i), :] = k32
                if n == 0 and hh == 0 and i in KT:
                    kvr[2][i - KT[0]] = _p32(_b16(k32).T)

        qs = {}

        def qnext(i):
            if i >= 0:
                if i not in qs:
                    qs[i] = qload(i)
                qstore(wq_n, i)

        qs[NB - 1] = qload(NB - 1)
        prev = None
        for i in range(NB - 1, -1, -1):
            top = i == NB - 1
            s_a = scores(qs[i], kvr, 0, i, top)
            if top:
                qnext(i)
            elif i == NB - 2:
                kvhalf(i + 1, 0)
                qnext(i - 1)
            else:
                qnext(i - 1)
                kvhalf(i + 1, 0)
            c_a = pv(s_a, kvr, 0, 2, True)
            s_b = scores(qs[i], kvr, 1, i)
            if top:
                qnext(i - 1)
            elif i in (NB - 2, 0):
                oproj(prev, i + 1)
                kvhalf(i + 1, 1)
            else:
                kvhalf(i + 1, 1)
                oproj(prev, i + 1)
            c_b = pv(s_b, kvr, 1, 3 if top else 2, True)
            prev = _cat1(c_a, c_b)
        kvproj(wkv_n, kvr, 0)
        oproj(prev, 0)
        for n in range(2):
            r0 = pl.multiple_of(jnp.minimum(j * 64, LAST0 // 2), 32)
            gu_t[j, n] = _p32(_b16(gu_buf[n, pl.ds(r0, 64), :]).T)

        nm = jnp.clip(j - 2, 0, 9)
        c0 = pl.multiple_of(jnp.where(j >= 2, 2 * M + 256 * nm, 0), 256)
        wm = _b16(wmod_buf[:, pl.ds(c0, 256)]).astype(f32)
        sct = sct_ref[...]
        pm = wm * _cat1(sct, sct)
        am = pm[0:8]
        for g in range(1, M // 8):
            am = am + pm[8 * g:8 * g + 8]
        mod_ref[jnp.where(j >= 2, nm, 10)] = am

        wq_cp(j + 2).wait()

        @pl.when(j == 1)
        def _():
            modb_cp().wait()

        @pl.when(j == 0)
        def _():
            for c_ in [wo_cp(1)] + gu_cp(1):
                c_.wait()

        @pl.when(j + 3 < NP)
        def _():
            for c_ in wkv_cp(j + 3):
                c_.wait()
        return carry

    def final():
        ja, jb = NP - 2, NP - 1
        for c_ in late_cps():
            c_.wait()
        wq15 = get_wq(jb)
        kvrs = (kv_refs(ja), kv_refs(jb))
        wo2 = _cat0(get_wo(ja), get_wo(jb))
        mods = {}
        wr1 = wr_buf[...].astype(f32).reshape(1, M)
        sub8 = lax.broadcasted_iota(i32, (8, 128), 0)
        lane8 = lax.broadcasted_iota(i32, (8, 128), 1)
        mod = _bf(jnp.sum(jnp.concatenate([mod_ref[n] for n in range(10)], axis=1), axis=0, keepdims=True))
        mods['ga'] = mod[:, 0:M]
        mods['sb'] = mod[:, M:2 * M]
        mods['cb1'] = _bf(1.0 + mod[:, 2 * M:3 * M])
        mods['gb'] = mod[:, 3 * M:4 * M]
        mods['gc'] = mods['gb'] * mods['cb1']
        mods['gs'] = mods['gb'] * mods['sb']
        mods['wc'] = wr1 * mods['cb1']
        mods['r0'] = jnp.sum(wr1 * mods['sb'], axis=-1, keepdims=True)

        cols = []
        state = [(-(2 ** 27)) + sub8]
        done_rows = {}

        def subsum(v, op):
            for sh in (4, 2, 1):
                v = op(v, pltpu.roll(v, sh, 0))
            return v

        def tree(vs, op):
            while len(vs) > 1:
                vs = [op(vs[k], vs[k + 1]) if k + 1 < len(vs) else vs[k] for k in range(0, len(vs), 2)]
            return vs[0]

        def merge(pend):
            kc = jnp.concatenate(pend, axis=0)
            st = state[0]
            gs = [kc[8 * g:8 * g + 8] for g in range(16)]
            r1 = subsum(tree([kg & eye_ref[8 * g:8 * g + 8, :] for g, kg in enumerate(gs)], jnp.bitwise_or),
                        jnp.bitwise_or)
            r2 = jnp.where(lane8 < 8, subsum(st & eye_ref[0:8, :], jnp.bitwise_or), -(2 ** 28))
            hi = 0.0
            lo = 0.0
            for rr in (r1, r2):
                cnt = tree([(rr - kg) >> 31 for kg in gs + [st]], jnp.add)
                sel = subsum(cnt, jnp.add) + sub8 == 0
                hi = hi + jnp.where(sel, (rr >> 11).astype(f32), 0.0)
                lo = lo + jnp.where(sel, (rr & 2047).astype(f32), 0.0)
            hi = _bc(jnp.sum(hi, axis=-1, keepdims=True)).astype(i32)
            lo = _bc(jnp.sum(lo, axis=-1, keepdims=True)).astype(i32)
            state[0] = (hi << 11) | lo
            return pltpu.bitcast(state[0], u32)

        deferred = []

        def emit_out(r0, x1, xc, rstd):
            of = x1 + (xc * _rep(rstd)) * mods['gc'] + mods['gs']
            out_buf[r0:r0 + PR, :] = of.astype(bf16)
            blk = r0 // TQ
            done_rows[blk] = done_rows.get(blk, 0) + PR
            if done_rows[blk] == TQ:
                out_cp(blk).start()
            return of

        def piece(r0):
            rel = yield
            x1 = acc_ref[r0:r0 + PR, :]
            sm = _bc(jnp.sum(_gate(x1, rel), axis=-1, keepdims=True))
            rel = yield
            m = _gate(sm, rel) * (1.0 / M)
            xc = x1 - _rep(m)
            sv = _bc(jnp.sum(xc * xc, axis=-1, keepdims=True))
            rw = _bc(jnp.sum(xc * mods['wc'], axis=-1, keepdims=True))
            rel = yield
            rstd = lax.rsqrt(_gate(sv, rel) * (1.0 / M) + EPS)
            st_ref[r0:r0 + PR, :] = _cat1(m, rstd)
            if r0 < S - TQ:
                dep = _bits(emit_out(r0, x1, xc, rstd))
            else:
                deferred.append((r0, m, rstd))
                dep = None
            r = _bf(rw * rstd + mods['r0'])
            rb = pltpu.bitcast(r, i32) >> 16
            rb = rb ^ ((rb >> 31) & 0x7FFF)
            idx = (S - 1 - r0) - lax.broadcasted_iota(i32, (PR, 128), 0)
            key = (rb << 11) | idx
            cols.append(key)
            return _bits(key) if dep is None else dep | _bits(key)

        def merge_task(pend):
            rel = yield
            return merge([_gate(pend[0], rel)] + pend[1:])

        live = []
        anchors = []
        nxt = [0]
        stage_gap = 200
        stage_cost = (16, 16, 32, 160)

        def advance(ent, t, rel):
            try:
                ent[2].send(rel)
                ent[0] = t + stage_gap
                ent[1] += 1
            except StopIteration as e:
                anchors.append([t + (530 if ent[1] == 3 else 280), e.value])
                live.remove(ent)
                if len(cols) * PR == 128:
                    g = merge_task(list(cols))
                    del cols[:]
                    next(g)
                    live.insert(0, [t + stage_gap, 3, g])

        def post_impl(res, dur):
            for g in range(min(res.shape[0] // 16, dur // 16)):
                t = clock[0] + 16 * g
                if t < nxt[0]:
                    continue
                for ent in live:
                    if ent[0] <= t:
                        nxt[0] = t + stage_cost[ent[1]]
                        advance(ent, t, pltpu.bitcast(res[16 * g:16 * g + 8, 0:128], u32))
                        break

        def take_impl(ng):
            deps = {}
            for g in range(ng):
                t = clock[0] + 16 * g
                ready = [an for an in anchors if an[0] <= t]
                anchors[:] = [an for an in anchors if an[0] > t]
                for an in ready:
                    deps[g] = an[1] | deps[g] if g in deps else an[1]
            return deps

        def ofin(ctx, i, r0, r1, w):
            rs = slice(i * TQ + r0, i * TQ + r1)
            lhs = _anchor(ctx, take((r1 - r0) // 16))
            a = acc_ref[rs, :] + jnp.dot(lhs, w, preferred_element_type=f32)
            clock[0] += 5 * (r1 - r0) * w.shape[0] // 512
            x = _b16(x_buf[(i * TQ + r0) // 2:(i * TQ + r1) // 2, :]).astype(f32)
            acc_ref[rs, :] = x + mods['ga'] * a
            for r in range(i * TQ + r0, i * TQ + r1, PR):
                g = piece(r)
                next(g)
                live.append([clock[0] + 200, 0, g])

        def opart(ctx, i, r0, r1):
            rs = slice(i * TQ + r0, i * TQ + r1)
            lhs = _anchor(ctx[r0:r1], take((r1 - r0) // 16))
            acc_ref[rs, :] += jnp.dot(lhs, wo2[:2 * D], preferred_element_type=f32)
            clock[0] += 5 * (r1 - r0) // 2

        hooks.update(take=take_impl, post=post_impl, chunk=4)
        clock[0] = 0
        q15 = {}
        prev = None
        o1, o2, qs = 80, 192, 64
        for i in range(NB):
            q14 = qload(i)
            lastb = i == NB - 1
            oprev = lambda r0, r1: ofin(prev[r0:r1], i - 1, r0, r1, wo2)
            if i < 3:
                s_a = scores(q14, kvrs[0], 0, i)
                s_b = scores(q14, kvrs[0], 1, i)
                if i == 0:
                    q15[0] = qproj(wq15, 0)
                else:
                    oprev(0, 192)
                c_a = pv(s_a, kvrs[0], 0)
                c_b = pv(s_b, kvrs[0], 1)
                s_c = scores(q15[i], kvrs[1], 0, i)
                s_d = scores(q15[i], kvrs[1], 1, i)
                if i == 0:
                    q15[1] = qproj(wq15, 1)
                else:
                    oprev(192, TQ)
                    q15[i + 1] = qproj(wq15, i + 1)
                c_c = pv(s_c, kvrs[1], 0)
                c_d = pv(s_d, kvrs[1], 1)
            else:
                s_a = scores(q14, kvrs[0], 0, i)
                oprev(0, o1)
                c_a = pv(s_a, kvrs[0], 0)
                s_b = scores(q14, kvrs[0], 1, i)
                oprev(o1, o2)
                c_b = pv(s_b, kvrs[0], 1)
                s_c = scores(q15[i], kvrs[1], 0, i)
                oprev(o2, TQ)
                if lastb:
                    c_ab = _cat1(c_a, c_b)
                    opart(c_ab, i, 0, qs)
                else:
                    qa = qproj(wq15, i + 1, 0, qs)
                c_c = pv(s_c, kvrs[1], 0)
                s_d = scores(q15[i], kvrs[1], 1, i)
                if lastb:
                    opart(c_ab, i, qs, TQ)
                    break
                q15[i + 1] = _cat0(qa, qproj(wq15, i + 1, qs, TQ))
                c_d = pv(s_d, kvrs[1], 1)
            prev = _cat1(c_a, c_b, c_c, c_d)
        hooks.update(take=None, post=None)
        rq = 64
        parts = []
        tok = None
        for k in range(TQ // rq + 2):
            if k < TQ // rq:
                part, tok = pv_rows(s_d, kvrs[1], 1, k * rq, (k + 1) * rq, tok)
                parts.append(part)
            if k >= 2:
                r0, r1 = (k - 2) * rq, (k - 1) * rq
                ofin(_cat1(c_c[r0:r1], parts[k - 2]), NB - 1, r0, r1, wo2[2 * D:])
        while live:
            advance(live[0], 0, None)
        assert not cols

        gb, cb1, sb = mods['gb'], mods['cb1'], mods['sb']
        sel = (S - 1) - (state[0] & 2047)
        sel_idx = [sel[t, 0] for t in range(C)]
        x1s = jnp.concatenate([acc_ref[pl.ds(it, 1), :] for it in sel_idx], axis=0)
        sts = jnp.concatenate([st_ref[pl.ds(it, 1), :] for it in sel_idx], axis=0)
        xn = (x1s - _rep(sts[:, :128])) * _rep(sts[:, 128:])
        xsb = (xn * cb1 + sb).astype(bf16)
        xs = xsb.astype(f32)
        rs = _bf(jnp.sum(xs * wr1, axis=-1, keepdims=True))
        wg = jnp.concatenate([_b16(gu_t[st, 0]) for st in range(NST)], axis=1)
        wu = jnp.concatenate([_b16(gu_t[st, 1]) for st in range(NST)], axis=1)
        g = jnp.dot(xsb, wg, preferred_element_type=f32)
        u = jnp.dot(xsb, wu, preferred_element_type=f32)
        toks = [pltpu.bitcast(t, u32) for t in _tiles(g)]
        for k, (r0, m, rstd) in enumerate(deferred):
            x1 = acc_ref[r0:r0 + PR, :]
            emit_out(r0, x1, x1 - _rep(_gate(m, toks[k // 3])), rstd)
        g = _bf(g)
        g = _bf(g * jax.nn.sigmoid(g))
        gu = g * _bf(u)
        nmain = (NST - 1) * 128
        dup = nmain - LAST0
        gu = _cat1(gu[:, :nmain], jnp.where(lane8 >= dup, gu[:, nmain:], 0.0))
        wd = _cat0(_b16(wd_buf[0:nmain // 2, :]), _b16(wd_buf[LAST0 // 2:F // 2, :]))
        y = _bf(jnp.dot(gu.astype(bf16), wd, preferred_element_type=f32))
        y = _bf(y * _bf(jax.nn.sigmoid(rs)))
        newrows = x1s + _bf(gb * _bf(xs + y))

        for i in range(NB):
            out_cp(i).wait()
        sub = lax.broadcasted_iota(i32, (8, M), 0)
        bases = []
        for t in range(C):
            it = sel_idx[t]
            base = pl.multiple_of((it >> 3) << 3, 8)
            bases.append(base)
            cur = out_buf[pl.ds(base, 8), :].astype(f32)
            out_buf[pl.ds(base, 8), :] = jnp.where(sub == (it & 7), newrows[t:t + 1, :], cur).astype(bf16)

        def fix_cp(t):
            return cp(out_buf.at[pl.ds(bases[t], 8), :], out_hbm.at[pl.ds(bases[t], 8), :], SEM_FIX + t)

        uniq = []
        for t in range(C):
            u_ = jnp.bool_(True)
            for t2 in range(t):
                u_ = jnp.logical_and(u_, bases[t] != bases[t2])
            uniq.append(u_)
        for t in range(C):
            pl.when(uniq[t])(lambda t=t: fix_cp(t).start())
        for t in range(C):
            pl.when(uniq[t])(lambda t=t: fix_cp(t).wait())

    prologue()
    lax.fori_loop(0, NP - 2, body, 0)
    final()


@jax.jit
def pallas_adaLN_cond__compressed_kv_cla__moe_arch_mod__prompt_kernel(
    A_x: jax.Array,
    A_c_kv: jax.Array,
    A_w_q: jax.Array,
    A_w_uk: jax.Array,
    A_w_uv: jax.Array,
    A_w_o: jax.Array,
    B_x: jax.Array,
    B_w_r: jax.Array,
    B_w_gate: jax.Array,
    B_w_up: jax.Array,
    B_w_down: jax.Array,
    c: jax.Array,
    w_mod: jax.Array,
):
    x = A_x.reshape(S, M)
    ckv = A_c_kv.reshape(S, DC)
    wo = A_w_o.reshape(H * D, M)
    hbm = pl.BlockSpec(memory_space=pltpu.HBM)

    out = pl.pallas_call(
        _kernel,
        in_specs=[hbm] * 12,
        out_specs=hbm,
        out_shape=jax.ShapeDtypeStruct((S, M), bf16),
        scratch_shapes=[
            pltpu.VMEM((S // 2, M), u32),
            pltpu.VMEM((S // 2, DC), u32),
            pltpu.VMEM((S // 2, M), u32),
            pltpu.VMEM((S, M), f32),
            pltpu.VMEM((2, 2, S // 2, D), u32),
            pltpu.VMEM((2, 2, S // 2, D), u32),
            pltpu.VMEM((S // 2, 2 * D), u32),
            pltpu.VMEM((4, M, D), u32),
            pltpu.VMEM((4, DC, D), u32),
            pltpu.VMEM((4, DC, D), u32),
            pltpu.VMEM((NP * D, M), u32),
            pltpu.VMEM((M // 2, 6 * M), u32),
            pltpu.VMEM((1, M), bf16),
            pltpu.VMEM((M,), bf16),
            pltpu.VMEM((2, F // 2, M), u32),
            pltpu.VMEM((NST, 2, M // 2, 128), u32),
            pltpu.VMEM((F // 2, M), u32),
            pltpu.VMEM((S, M), bf16),
            pltpu.VMEM((HB, HB), i32),
            pltpu.VMEM((S, 256), f32),
            pltpu.VMEM((2, 2, D // 2, TQ), u32),
            pltpu.VMEM((M, 128), f32),
            pltpu.VMEM((11, 8, 256), f32),
            pltpu.SemaphoreType.DMA((NSEM,)),
        ],
        compiler_params=pltpu.CompilerParams(
            vmem_limit_bytes=100 * 1024 * 1024,
            disable_bounds_checks=True,
            disable_semaphore_checks=True,
        ),
    )(x, ckv, A_w_q, A_w_uk, A_w_uv, wo, B_w_r, B_w_gate.T, B_w_up.T, B_w_down, c, w_mod)
    return out.reshape(1, S, M)
```
